```python
import jax
import jax.numpy as jnp

def _softmax(x, axis=-1):
    return jax.nn.softmax(x, axis=axis)
def _gelu(x):
    return jax.nn.gelu(x, approximate=True)
def _silu(x):
    return jax.nn.silu(x)
def _sigmoid(x):
    return jax.nn.sigmoid(x)
def _layernorm(x, axis=-1, eps=1e-5):
    m = jnp.mean(x, axis=axis, keepdims=True)
    v = jnp.var(x, axis=axis, keepdims=True)
    return (x - m) / jnp.sqrt(v + eps)
def _scatter_add(tgt, idx, src, axis=0):
    return tgt.at[idx].add(src)
def _segment_sum(src, seg, n):
    return jax.ops.segment_sum(src, seg, n)
class _Rng:
    def __init__(self, key):
        self._k = key
    def _next(self):
        self._k, sub = jax.random.split(self._k)
        return sub
    def normal(self, shape):
        return jax.random.normal(self._next(), shape, dtype=jnp.bfloat16)
    def randint(self, lo, hi, shape):
        return jax.random.randint(self._next(), shape, lo, hi, dtype=jnp.int32)
    def uniform(self, shape, lo=0.0, hi=1.0):
        return jax.random.uniform(self._next(), shape, jnp.bfloat16, lo, hi)
    def permutation(self, n):
        return jax.random.permutation(self._next(), n)


kernel_name = 'parallel_sum__compressed_kv_cla__moe_arch_mod__prompt'

def _fwd_setup_inputs():
    _rng = _Rng(jax.random.key(int.from_bytes(__import__("os").urandom(4), "little")))
    _w = (lambda a: (lambda t: t.astype(jnp.bfloat16) if jnp.issubdtype(t.dtype, jnp.floating) else t)(jnp.asarray(a)))
    def _A_setup():
        B, H, Sq, Sk, D, M = 1, 32, 2048, 2048, 128, 576
        Dc = 4 * D
        return {
            "x": _w((lambda *s: _rng.normal(s) * 0.05)(B, Sq, M)),
            "c_kv": _w((lambda *s: _rng.normal(s) * 0.05)(B, Sk, Dc)),
            "w_q": _w((lambda *s: _rng.normal(s) * 0.05)(M, H, D) * (M ** -0.5)),
            "w_uk": _w((lambda *s: _rng.normal(s) * 0.05)(Dc, H, D) * (Dc ** -0.5)),
            "w_uv": _w((lambda *s: _rng.normal(s) * 0.05)(Dc, H, D) * (Dc ** -0.5)),
            "w_o": _w((lambda *s: _rng.normal(s) * 0.05)(H, D, M) * ((H * D) ** -0.5)),
        }
    _A_in = _A_setup()

    def _B_setup():
        B, S, D, F, C = 1, 2048, 576, 4608, 8
        return {
            "x": _w((lambda *s: _rng.normal(s) * 0.05)(B, S, D)),
            "w_r": _w((lambda *s: _rng.normal(s) * 0.05)(D)),
            "w_gate": _w((lambda *s: _rng.normal(s) * 0.05)(D, F)),
            "w_up": _w((lambda *s: _rng.normal(s) * 0.05)(D, F)),
            "w_down": _w((lambda *s: _rng.normal(s) * 0.05)(F, D)),
        }
    _B_in = _B_setup()

    return {
        "A_x": _A_in["x"],
        "A_c_kv": _A_in["c_kv"],
        "A_w_q": _A_in["w_q"],
        "A_w_uk": _A_in["w_uk"],
        "A_w_uv": _A_in["w_uv"],
        "A_w_o": _A_in["w_o"],
        "B_x": _B_in["x"],
        "B_w_r": _B_in["w_r"],
        "B_w_gate": _B_in["w_gate"],
        "B_w_up": _B_in["w_up"],
        "B_w_down": _B_in["w_down"],
    }

def _fwd_reference(A_x, A_c_kv, A_w_q, A_w_uk, A_w_uv, A_w_o, B_x, B_w_r, B_w_gate, B_w_up, B_w_down):
    def _A_ref(x, c_kv, w_q, w_uk, w_uv, w_o):
        B, Sq, M = x.shape[0], x.shape[1], x.shape[2]
        Sk = c_kv.shape[1]
        H, D = w_q.shape[1], w_q.shape[2]
        q = jnp.einsum("bqm,mhd->bhqd", x, w_q)
        k = jnp.einsum("bkc,chd->bhkd", c_kv, w_uk)
        v = jnp.einsum("bkc,chd->bhkd", c_kv, w_uv)
        scores = jnp.einsum("bhqd,bhkd->bhqk", q, k) * (D ** -0.5)
        off = Sk - Sq
        qi = jnp.arange(Sq)[:, None]
        kj = jnp.arange(Sk)[None, :]
        cmask = kj <= (qi + off)
        scores = jnp.where(cmask[None, None], scores, -1e9)
        p = _softmax(scores, axis=-1)
        ctx = jnp.einsum("bhqk,bhkd->bhqd", p, v)
        return jnp.einsum("bhqd,hdm->bqm", ctx, w_o)

    def _B_ref(x, w_r, w_gate, w_up, w_down):
        B, S, D = x.shape
        C = 8
        r = x @ w_r
        idx = jnp.argsort(jax.lax.stop_gradient(-r), axis=-1)[:, :C]
        idx_e = jnp.repeat(idx.reshape(B, C, 1), D, axis=2)
        x_sel = jnp.take_along_axis(x, idx_e, axis=1)
        g = _silu(x_sel @ w_gate)
        u = x_sel @ w_up
        y = (g * u) @ w_down
        r_sel = _sigmoid(jnp.take_along_axis(r, idx, axis=1))
        y = y * r_sel.reshape(B, C, 1)
        b_off = (jnp.arange(B) * S).reshape(B, 1)
        flat_idx = (idx + b_off).reshape(B * C)
        zero = (x * 0.0).reshape(B * S, D)
        upd = _scatter_add(zero, flat_idx, y.reshape(B * C, D), axis=0)
        return x + upd.reshape(B, S, D)

    x = A_x
    xn = _layernorm(x, axis=-1)
    return x + _A_ref(xn, A_c_kv, A_w_q, A_w_uk, A_w_uv, A_w_o) + _B_ref(xn, B_w_r, B_w_gate, B_w_up, B_w_down)


def setup_inputs():
    _inp = _fwd_setup_inputs()
    _gk = jax.random.fold_in(jax.random.key(int.from_bytes(__import__("os").urandom(4), "little")), 2**31 - 1)
    _shapes = [[1, 2048, 576]]
    _dtypes = ['bfloat16']
    _gks = jax.random.split(_gk, len(_shapes))
    _gs = [jax.random.normal(k, s, dtype=jnp.dtype(d)) * 0.05 for k, s, d in zip(_gks, _shapes, _dtypes)]
    _inp["grad_out"] = _gs[0]
    return _inp

def reference(A_x, A_c_kv, A_w_q, A_w_uk, A_w_uv, A_w_o, B_w_r, B_w_gate, B_w_up, B_w_down, B_x, grad_out):
    _const = dict(B_x=B_x)
    def _f(*_d):
        return _fwd_reference(**{'A_x': _d[0], 'A_c_kv': _d[1], 'A_w_q': _d[2], 'A_w_uk': _d[3], 'A_w_uv': _d[4], 'A_w_o': _d[5], 'B_w_r': _d[6], 'B_w_gate': _d[7], 'B_w_up': _d[8], 'B_w_down': _d[9], **_const})
    _out, _vjp = jax.vjp(_f, A_x, A_c_kv, A_w_q, A_w_uk, A_w_uv, A_w_o, B_w_r, B_w_gate, B_w_up, B_w_down)
    _grads = _vjp(grad_out)
    _out0 = jnp.asarray(_out)
    return (_out0, *[jnp.asarray(_g) for _g in _grads])
```

```python
import functools, math
import jax
import jax.numpy as jnp
from jax import lax
import jax.experimental.pallas as pl
import jax.experimental.pallas.tpu as pltpu

f32 = jnp.float32
bf16 = jnp.bfloat16
NN = (((1,), (0,)), ((), ()))
NT = (((1,), (1,)), ((), ()))
TN = (((0,), (0,)), ((), ()))

S, M, DC, H, D, F, C = 2048, 576, 512, 32, 128, 4608, 8
HG = 8
FC = 256
NF = F // FC
TB = 512
CP = 16
EPS = 1e-5
EPS_BF16 = 1.0013580322265625e-05
LOG2E = 1.4426950408889634
LN2 = 0.6931471805599453
SCALE = D ** -0.5
NEG = -1e30


def dot(a, b, dims=NN):
    return lax.dot_general(a, b, dims, preferred_element_type=f32)


def rb(x):
    return x.astype(bf16).astype(f32)


def ln_stats(xf, axis):
    mean = jnp.sum(xf, axis=axis, keepdims=True) * (1.0 / M)
    xc = xf - mean
    var = jnp.sum(xc * xc, axis=axis, keepdims=True) * (1.0 / M)
    sd = rb(jnp.sqrt(rb(rb(var) + EPS_BF16)))
    xn = (rb(xf - rb(mean)) / sd).astype(bf16)
    rstd = lax.rsqrt(var + EPS)
    return xn, rstd


def make_kernel(CH=32, LAG=256, FORCE=False, DSPLIT=2048):

  def kernel(x_ref, c_ref, g_ref, wq_ref, wuk_ref, wuv_ref, wo_ref, wr_ref, wg_ref, wu_ref, wd_ref,
           out_ref, dx_ref, dc_ref, dwq_ref, dwuk_ref, dwuv_ref, dwo_ref, dwr_ref, dwg_ref, dwu_ref, dwd_ref,
           xnT_s, gT_s, cT_s, c_s, rstd_s, r_s, outT_a, dxnT_a, dc_a,
           wq_s, wkv_s, dwq_s, dwkv_s,
           qT_s, k_s, kT_s, v_s, vT_s, doT_s, ctxT_s, dqT_s, dob_s, dkv_s, wqT_s, wo_s,
           z_s, s_s, p_s, ds_s,
           oh_s, xs_s, dy0_s, xsT_s, dy_s, rs_s, y0_a, dxs_a):
    h = pl.program_id(0)
    hh = h % HG

    @pl.when(h == 0)
    def _():
        for i in range(4):
            z_s[i] = i % 2
        wr = wr_ref[...].reshape(1, M)
        wr16 = jnp.broadcast_to(wr, (CP, M))

        def body(i, carry):
            o = pl.multiple_of(i * TB, TB)
            rows = pl.ds(o, TB)
            xf = x_ref[:, rows].astype(f32)
            xn, rstd = ln_stats(xf, 0)
            xnT_s[:, rows] = xn
            rstd_s[:, rows] = rstd
            outT_a[:, rows] = xf + xn.astype(f32)
            r_s[:, rows] = dot(wr16, xn)
            gT = g_ref[:, rows]
            gT_s[:, rows] = gT
            dxnT_a[:, rows] = gT.astype(f32)
            cb = c_ref[rows, :]
            c_s[rows, :] = cb
            cT_s[:, rows] = cb.T
            dc_a[rows, :] = jnp.zeros((TB, DC), f32)
            return carry

        lax.fori_loop(0, S // TB, body, 0)

        r = rb(r_s[0:C, :])
        bits = pltpu.bitcast(r, jnp.int32)
        mono = jnp.where(bits >= 0, bits, -(bits & 0x7FFFFFFF))
        key = mono + (0xFFFF - lax.broadcasted_iota(jnp.int32, (C, S), 1))
        sub = lax.broadcasted_iota(jnp.int32, (C, S), 0)
        oh = jnp.zeros((C, S), f32)
        for c in range(C):
            hit = key == jnp.max(key, axis=1, keepdims=True)
            key = jnp.where(hit, jnp.int32(-2 ** 31), key)
            oh = jnp.where(hit & (sub == c), 1.0, oh)
        rsel = jnp.sum(jnp.where(oh > 0.0, r, 0.0), axis=1, keepdims=True)
        rs = jax.nn.sigmoid(rsel)
        rs = jnp.concatenate([rs, rs], axis=0)
        oh_s[...] = jnp.concatenate([oh, oh], axis=0).astype(bf16)
        oh0 = jnp.concatenate([oh, jnp.zeros((C, S), f32)], axis=0).astype(bf16)
        xs = dot(oh0, xnT_s[...], NT)
        dy = dot(oh0, gT_s[...], NT)
        dy0 = rb(dy * rs)
        xs_s[...] = xs.astype(bf16)
        dy0_s[...] = dy0.astype(bf16)
        dy_s[...] = dy
        xsT_s[...] = jnp.concatenate([xs, dy0, jnp.zeros((128 - 2 * CP, M), f32)], axis=0).T.astype(bf16)
        rs_s[...] = jnp.broadcast_to(rs, (CP, 128))
        y0_a[...] = jnp.zeros((CP, M), f32)
        dxs_a[...] = jnp.zeros((CP, M), f32)

    @pl.when(hh == 0)
    def _():
        wq = wq_ref[...].reshape(M, HG * D)
        wk = wuk_ref[...].reshape(DC, HG * D)
        wv = wuv_ref[...].reshape(DC, HG * D)
        for j in range(HG):
            wq_s[j] = wq[:, j * D:(j + 1) * D]
            wkv_s[j, :, 0:D] = wk[:, j * D:(j + 1) * D]
            wkv_s[j, :, D:2 * D] = wv[:, j * D:(j + 1) * D]

    @pl.when(h < NF)
    def _():
        xs = xs_s[...]
        dy0 = dy0_s[...]
        wg = wg_ref[...]
        wu = wu_ref[...]
        wd = wd_ref[...]
        a = dot(xs, wg)
        u = dot(xs, wu)
        dh = dot(dy0, wd)
        sg = jax.nn.sigmoid(a)
        gl = a * sg
        hb = (gl * u).astype(bf16)
        du = (dh * gl).astype(bf16)
        da = (dh * u * (sg * (1.0 + a * (1.0 - sg)))).astype(bf16)
        y0_a[...] += dot(hb, wd, NT)
        dxs_a[...] += dot(da, wg, NT) + dot(du, wu, NT)
        zero = jnp.zeros((CP, FC), bf16)
        lhs = xsT_s[:, 0:2 * CP]
        dwg_ref[...] = dot(lhs, jnp.concatenate([da, zero], axis=0)).astype(bf16)
        dwu_ref[...] = dot(lhs, jnp.concatenate([du, zero], axis=0)).astype(bf16)
        dwd_ref[...] = dot(lhs, jnp.concatenate([zero, hb], axis=0)).astype(bf16)

    T = 128
    NT_ = S // T
    wq = wq_s[hh]
    wkv = wkv_s[hh]
    woT = wo_ref[...]
    wqT_s[...] = wq.T
    wo_s[...] = woT.T
    zw = [z_s[0], z_s[1]]
    zr = [z_s[2], z_s[3]]
    tri = (lax.broadcasted_iota(jnp.int32, (T, T), 0) <= lax.broadcasted_iota(jnp.int32, (T, T), 1))
    tile = lambda j: slice(j * T, (j + 1) * T)
    span = lambda j0, j1: slice(j0 * T, j1 * T)
    st = {}

    def kproj(j0, j1):
        k = dot(c_s[span(j0, j1), :], wkv[:, 0:D]).astype(bf16)
        k_s[span(j0, j1), :] = k
        kT_s[:, span(j0, j1)] = k.T

    def vproj(j0, j1):
        v = dot(c_s[span(j0, j1), :], wkv[:, D:2 * D]).astype(bf16)
        v_s[span(j0, j1), :] = v
        vT_s[:, span(j0, j1)] = v.T

    def qproj(j0, j1):
        qT_s[:, span(j0, j1)] = (dot(wqT_s[...], xnT_s[:, span(j0, j1)]) * (SCALE * LOG2E)).astype(bf16)

    def doproj(j0, j1):
        doT_s[:, span(j0, j1)] = dot(wo_s[...], gT_s[:, span(j0, j1)])

    def a_b(ja, jb):
        na = (ja + 1) * T // CH if ja is not None else 0
        nb = (jb + 1) * T // CH if jb is not None else 0
        if ja is not None:
            s = dot(k_s[0:(ja + 1) * T, :], qT_s[:, tile(ja)])
        lag = min(LAG // CH, max(na - 1, 0))
        mx, l, done = None, None, 0
        for i in range(max(na, 1)):
            if ja is not None:
                si = s[i * CH:(i + 1) * CH, :]
                o = i * CH - ja * T
                if o >= 0:
                    si = jnp.where(tri[o:o + CH, :], si, NEG)
                s_s[zw[ja % 2], i * CH:(i + 1) * CH, :] = si
                mi = jnp.max(si.reshape(CH // 8, 8, T), axis=0)
                mx = mi if mx is None else jnp.maximum(mx, mi)
                if FORCE:
                    s_s[zw[ja % 2], S:S + 8, :] = mx
            if jb is not None:
                upto = nb if i == max(na, 1) - 1 else (0 if i < lag else ((i - lag + 1) * nb) // (na - lag))
                for u in range(done, upto):
                    r = slice(u * CH, (u + 1) * CH)
                    p = jnp.exp2(s_s[zr[jb % 2], r, :] - st['m', jb])
                    li = jnp.sum(p.reshape(CH // 8, 8, T), axis=0)
                    l = li if l is None else l + li
                    p_s[jb, r, :] = p.astype(bf16)
                done = upto
        if ja is not None:
            st['m', ja] = jnp.max(mx, axis=0, keepdims=True)
        if jb is not None:
            inv = 1.0 / jnp.sum(l, axis=0, keepdims=True)
            st['inv', jb] = inv
            dob_s[:, tile(jb)] = (doT_s[:, tile(jb)] * inv).astype(bf16)

    def c_(j):
        inv = st['inv', j]
        oT = dot(vT_s[:, 0:(j + 1) * T], p_s[j, 0:(j + 1) * T, :]) * inv
        ctxT_s[:, tile(j)] = oT.astype(bf16)
        st['delta', j] = jnp.sum(doT_s[:, tile(j)] * oT, axis=0, keepdims=True) * inv

    def d_(j):
        for r0 in range(0, (j + 1) * T, DSPLIT):
            r = slice(r0, min(r0 + DSPLIT, (j + 1) * T))
            dp = dot(v_s[r, :], dob_s[:, tile(j)])
            ds_s[j, r, :] = (p_s[j, r, :].astype(f32) * (dp - st['delta', j])).astype(bf16)

    def q_(j):
        dqT_s[:, tile(j)] = (dot(kT_s[:, 0:(j + 1) * T], ds_s[j, 0:(j + 1) * T, :]) * SCALE).astype(bf16)

    def v_(i):
        lhs = jnp.concatenate([p_s[j, tile(i), :] for j in range(NT_ - 1, i - 1, -1)], axis=1)
        rhs = jnp.concatenate([dob_s[:, tile(j)] for j in range(NT_ - 1, i - 1, -1)], axis=1)
        dkv_s[tile(i), D:2 * D] = dot(lhs, rhs, NT).astype(bf16)

    def k_(i):
        lhs = jnp.concatenate([ds_s[j, tile(i), :] for j in range(NT_ - 1, i - 1, -1)], axis=1)
        rhs = jnp.concatenate([qT_s[:, tile(j)] for j in range(NT_ - 1, i - 1, -1)], axis=1)
        dkv_s[tile(i), 0:D] = (dot(lhs, rhs, NT) * LN2).astype(bf16)

    def acc(name, val):
        st[name] = val if name not in st else st[name] + val

    def post_o(j0, j1):
        ctxT = ctxT_s[:, span(j0, j1)]
        outT_a[:, span(j0, j1)] += dot(woT, ctxT)
        acc('dwo', dot(gT_s[:, span(j0, j1)], ctxT, NT))

    def post_q(j0, j1):
        dqT = dqT_s[:, span(j0, j1)]
        dxnT_a[:, span(j0, j1)] += dot(wq, dqT)
        acc('dwq', dot(xnT_s[:, span(j0, j1)], dqT, NT))

    def post_kv(j0, j1):
        dkv = dkv_s[span(j0, j1), :]
        dc_a[span(j0, j1), :] += dot(dkv, wkv, NT)
        acc('dwkv', dot(cT_s[:, span(j0, j1)], dkv))

    for b in range(4):
        kproj(4 * b, 4 * b + 4)
    qproj(12, 16)
    for t in range(NT_ + 4):
        j = NT_ - 1 - t
        ok = lambda x: 0 <= x < NT_
        if t == 0:
            doproj(12, 16)
        if ok(j) or ok(j + 1):
            a_b(j if ok(j) else None, j + 1 if ok(j + 1) else None)
        if t == 0:
            vproj(0, 4); vproj(4, 8); vproj(8, 12)
        if t == 1:
            vproj(12, 16); qproj(8, 12); doproj(8, 12)
        if ok(j + 3):
            d_(j + 3)
        if ok(j + 2):
            c_(j + 2)
        if t == 2:
            qproj(4, 8); doproj(4, 8)
        if t == 3:
            qproj(0, 4); doproj(0, 4)
        if ok(j + 2):
            v_(j + 2)
        if ok(j + 4):
            q_(j + 4)
            k_(j + 4)
    for b in range(3, -1, -1):
        post_o(4 * b, 4 * b + 4)
        post_q(4 * b, 4 * b + 4)
        post_kv(4 * b, 4 * b + 4)
    dwq_s[hh] = st['dwq'].astype(bf16)
    dwkv_s[hh] = st['dwkv'].astype(bf16)
    dwo_ref[...] = st['dwo'].astype(bf16)

    @pl.when(hh == HG - 1)
    def _():
        dwq_ref[...] = jnp.concatenate([dwq_s[j] for j in range(HG)], axis=1).reshape(M, HG, D)
        dwuk_ref[...] = jnp.concatenate([dwkv_s[j, :, 0:D] for j in range(HG)], axis=1).reshape(DC, HG, D)
        dwuv_ref[...] = jnp.concatenate([dwkv_s[j, :, D:2 * D] for j in range(HG)], axis=1).reshape(DC, HG, D)

    @pl.when(h == H - 1)
    def _():
        rs = rs_s[0:C, 0:1]
        y0 = y0_a[0:C, :]
        xs = xs_s[...].astype(f32)[0:C, :]
        dr = jnp.sum(dy_s[0:C, :] * y0, axis=1, keepdims=True) * (rs * (1.0 - rs))
        dwr_ref[...] = jnp.sum(dr * xs, axis=0, keepdims=True).astype(bf16).reshape(M)
        y = y0 * rs
        de = dxs_a[0:C, :] + dr * wr_ref[...].reshape(1, M).astype(f32)
        yh, deh = rb(y), rb(de)
        eT = jnp.concatenate([yh, y - yh, deh, de - deh, jnp.zeros((128 - 4 * C, M), f32)], axis=0).T.astype(bf16)
        xsT_s[...] = eT

        def body(i, carry):
            o = pl.multiple_of(i * TB, TB)
            rows = pl.ds(o, TB)
            oh = oh_s[:, rows]
            zero = jnp.zeros((CP, TB), bf16)
            lhs = xsT_s[:, 0:2 * CP]
            out_ref[:, rows] = (outT_a[:, rows] + dot(lhs, jnp.concatenate([oh, zero], axis=0))).astype(bf16)
            dn = dxnT_a[:, rows] + dot(lhs, jnp.concatenate([zero, oh], axis=0))
            xh = xnT_s[:, rows].astype(f32)
            m1 = jnp.sum(dn, axis=0, keepdims=True) * (1.0 / M)
            m2 = jnp.sum(dn * xh, axis=0, keepdims=True) * (1.0 / M)
            dxT = gT_s[:, rows].astype(f32) + (dn - m1 - xh * m2) * rstd_s[:, rows]
            dx_ref[:, rows] = dxT.astype(bf16)
            dc_ref[rows, :] = dc_a[rows, :].astype(bf16)
            return carry

        lax.fori_loop(0, S // TB, body, 0)

  return kernel


def build(**kw):
  kernel = make_kernel(**kw)

  @jax.jit
  def fn(A_x, A_c_kv, A_w_q, A_w_uk, A_w_uv, A_w_o, B_x, B_w_r, B_w_gate, B_w_up, B_w_down, grad_out):
    one = pl.Buffered(1)
    const = lambda shape: pl.BlockSpec(shape, lambda h: (0,) * len(shape), pipeline_mode=one)
    consto = lambda shape: pl.BlockSpec(shape, lambda h: (0,) * len(shape))
    grp = lambda n: pl.BlockSpec((n, HG, D), lambda h: (0, h // HG, 0))
    fcol = pl.BlockSpec((M, FC), lambda h: (0, jnp.minimum(h, NF - 1)))
    frow = pl.BlockSpec((FC, M), lambda h: (jnp.minimum(h, NF - 1), 0))
    wob = pl.BlockSpec((None, M, D), lambda h: (h, 0, 0))
    in_specs = [const((M, S)), const((S, DC)), const((M, S)), grp(M), grp(DC), grp(DC), wob, const((M,)), fcol, fcol, fcol]
    out_specs = [consto((M, S)), consto((M, S)), consto((S, DC)), grp(M), grp(DC), grp(DC), wob, consto((M,)), fcol, fcol, fcol]
    sds = lambda *s: jax.ShapeDtypeStruct(s, bf16)
    out_shape = [sds(M, S), sds(M, S), sds(S, DC), sds(M, H, D), sds(DC, H, D), sds(DC, H, D), sds(H, M, D), sds(M), sds(M, F), sds(M, F), sds(M, F)]
    V = pltpu.VMEM
    scratch = [
        V((M, S), bf16), V((M, S), bf16), V((DC, S), bf16), V((S, DC), bf16), V((1, S), f32), V((CP, S), f32),
        V((M, S), f32), V((M, S), f32), V((S, DC), f32),
        V((HG, M, D), bf16), V((HG, DC, 2 * D), bf16), V((HG, M, D), bf16), V((HG, DC, 2 * D), bf16),
        V((D, S), bf16), V((S, D), bf16), V((D, S), bf16), V((S, D), bf16), V((D, S), bf16), V((D, S), f32),
        V((D, S), bf16), V((D, S), bf16), V((D, S), bf16), V((S, 2 * D), bf16), V((D, M), bf16), V((D, M), bf16),
        pltpu.SMEM((4,), jnp.int32), V((2, S + 8, 128), f32), V((16, S, 128), bf16), V((16, S, 128), bf16),
        V((CP, S), bf16), V((CP, M), bf16), V((CP, M), bf16), V((M, 128), bf16), V((CP, M), f32), V((CP, 128), f32),
        V((CP, M), f32), V((CP, M), f32),
    ]
    outs = pl.pallas_call(
        kernel, grid=(H,), in_specs=in_specs, out_specs=out_specs, out_shape=out_shape, scratch_shapes=scratch,
        compiler_params=pltpu.CompilerParams(dimension_semantics=("arbitrary",), vmem_limit_bytes=120 * 2 ** 20),
        name="fused_kernel",
    )(A_x.reshape(S, M).T, A_c_kv.reshape(S, DC), grad_out.reshape(S, M).T, A_w_q, A_w_uk, A_w_uv, A_w_o.transpose(0, 2, 1),
      B_w_r, B_w_gate, B_w_up, B_w_down.T)
    out, dx, dc, dwq, dwuk, dwuv, dwo, dwr, dwg, dwu, dwd = outs
    return (out.T.reshape(1, S, M), dx.T.reshape(1, S, M), dc.reshape(1, S, DC), dwq, dwuk, dwuv, dwo.transpose(0, 2, 1), dwr, dwg, dwu, dwd.T)

  return fn


_fn = build()


@jax.jit
def pallas_parallel_sum__compressed_kv_cla__moe_arch_mod__prompt_kernel(
    A_x: jax.Array,
    A_c_kv: jax.Array,
    A_w_q: jax.Array,
    A_w_uk: jax.Array,
    A_w_uv: jax.Array,
    A_w_o: jax.Array,
    B_x: jax.Array,
    B_w_r: jax.Array,
    B_w_gate: jax.Array,
    B_w_up: jax.Array,
    B_w_down: jax.Array,
    grad_out: jax.Array,
):
    return _fn(A_x, A_c_kv, A_w_q, A_w_uk, A_w_uv, A_w_o, B_x, B_w_r, B_w_gate, B_w_up, B_w_down, grad_out)
```

```python
import functools

import jax
import jax.numpy as jnp
from jax import lax
import jax.experimental.pallas as pl
import jax.experimental.pallas.tpu as pltpu

f32 = jnp.float32
bf16 = jnp.bfloat16
u32 = jnp.uint32
NN = (((1,), (0,)), ((), ()))
NT = (((1,), (1,)), ((), ()))

S, M, DC, H, D, F, C = 2048, 576, 512, 32, 128, 4608, 8
HG = 8
NG = H // HG
T = 128
NTL = S // T
TB = 2 * T
NB = S // TB
KH = 256
MR = M - 2 * KH
DH = D // 2
CP = 16
FX = F - H * T
EPS = 1e-5
EPS_BF16 = 1.0013580322265625e-05
LOG2E = 1.4426950408889634
LN2 = 0.6931471805599453
SCALE = D ** -0.5
NEG = -1e30


def dot(a, b, dims=NN):
    return lax.dot_general(a, b, dims, preferred_element_type=f32)


def rb(x):
    return x.astype(bf16).astype(f32)


def pk(x):
    return pltpu.bitcast(x.astype(bf16), u32)


def upk(u):
    return pltpu.bitcast(u, bf16)


def sum_a(a11, a12, a21, a22):
    return [a11 + a22, a21 + a22, a11, a22, a11 + a12, a21 - a11, a12 - a22]


def sum_b(b11, b12, b21, b22):
    return [b11 + b22, b11, b12 - b22, b21 - b11, b22, b11 + b12, b21 + b22]


def sum_c(c11, c12, c21, c22):
    return [c11 + c22, c21 - c22, c12 + c22, c11 + c21, c12 - c11, c22, c11]


def comb_c(m):
    return m[0] + m[3] - m[4] + m[6], m[2] + m[4], m[1] + m[3], m[0] - m[1] + m[2] + m[5]


def comb_a(m):
    return m[0] + m[2] + m[4] - m[5], m[4] + m[6], m[1] + m[5], m[0] + m[1] + m[3] - m[6]


def comb_b(m):
    return m[0] + m[1] - m[3] + m[5], m[2] + m[5], m[3] + m[6], m[0] - m[2] + m[4] + m[6]


def schedule(PT=(1, 0, -1, -2), V=1, NF=3, F=1, POST=2):
    seq = lambda op, t, rs: ["%s%d.%d" % (op, t, r) for r in rs] if 0 <= t < NB else []
    mix = lambda a, b: [x for pair in zip(a, b) for x in pair] if a and b else a + b
    out = ["K%d" % t for t in range(NB)] + ["Q7 Q6"]
    f = [("a15 a14 V0 V1 V2 V3 V4 Q5", "e7 a13 V5 V6 V7 T O7 O6 Q4 a12 O5 O4 O3 O2", "O1 O0", "Q3 Q2 Q1 Q0"),
         ("a15 a14 V0 V1 V2 V3 V4 V5", "e7 a13 V6 V7 T O7 O6 O5 a12 Q5 O4 O3 O2 O1", "Q4 O0", "Q3 Q2 Q1 Q0")][F]
    out += [f[0], f[1]]
    for t in range(5, -4, -1):
        if t + 1 >= 0:
            out.append("e%d" % (t + 1))
        if t >= 0:
            out.append("a%d" % (2 * t + 1))
            if V == 1:
                out.append("a%d" % (2 * t))
        out += seq("c", t + 2, range(8))
        if t == 5:
            out.append(f[2])
        out += mix(seq("n", t + 3, range(NF)), seq("m", t + 3, range(NF)))
        out += seq("d", t + 2, [2])
        if t >= 0 and V == 0:
            out.append("a%d" % (2 * t))
        if t == 5:
            out.append(f[3])
        out += seq("v", t + 2, range(8))
        out += mix(seq("n", t + 3, range(NF, 8)), seq("m", t + 3, range(NF, 8)))
        for n in range(4):
            if PT[n] == t:
                out.append("p%d" % n)
    out.append([
        "o0 o1 o2 o3 o4 o5 o6 o7 y3 y2 y1 y0 q0 q1 q2 q3 q4 q5 q6 q7 x3 x2 x1 x0 k0 k1 k2 k3 k4 k5 k6 "
        "g0 f0 g1 f1 g2 f2 g3 f3 g4 g5 g6 b0 g7 b1 g8 b2 g9 b3 w g10 g11 g12 g13",
        "o0 o1 o2 o3 o4 o5 o6 o7 y3 f0 y2 f1 y1 f2 y0 f3 q0 q1 q2 q3 q4 q5 q6 q7 W x3 b0 x2 b1 x1 b2 x0 b3 k0 k1 k2 k3 k4 k5 k6 "
        "g0 g1 g2 g3 g4 g5 g6 g7 g8 g9 g10 g11 g12 g13",
        "o0 o1 o2 o3 o4 o5 o6 o7 y3 f0 y2 f1 q0 q1 q2 q3 q4 q5 q6 q7 y1 f2 y0 f3 x3 W x2 b0 x1 b1 x0 b2 k0 b3 k1 k2 k3 k4 k5 k6 "
        "g0 g1 g2 g3 g4 g5 g6 g7 g8 g9 g10 g11 g12 g13",
        "o0 o1 o2 o3 o4 o5 o6 o7 y3 f0 y2 f1 q0 q1 q2 q3 q4 q5 q6 q7 y1 f2 y0 f3 x3 W x2 b0 x1 b1 x0 b2 p0 k0 b3 p1 k1 p2 k2 p3 k3 k4 k5 k6 "
        "g0 g1 g2 g3 g4 g5 g6 g7 g8 g9 g10 g11 g12 g13",
        "o0 o1 o2 o3 o4 o5 o6 o7 y3 f0 y2 f1 q0 q1 q2 q3 q4 q5 q6 q7 y1 f2 y0 f3 p0 x3 W x2 b0 p1 x1 b1 x0 b2 p2 k0 b3 k1 p3 k2 k3 k4 k5 k6 "
        "g0 g1 g2 g3 g4 g5 g6 g7 g8 g9 g10 g11 g12 g13",
        "o0 o1 y3 o2 o3 y2 o4 o5 y1 o6 o7 y0 q0 q1 x3 q2 q3 x2 q4 q5 x1 q6 q7 x0 k0 f0 k1 f1 k2 f2 k3 f3 k4 W k5 b0 k6 b1 "
        "g0 b2 g1 b3 g2 g3 g4 g5 g6 g7 g8 g9 g10 g11 g12 g13",
        "y3 f0 y2 f1 y1 f2 y0 f3 x3 W x2 b0 x1 b1 x0 o0 o1 k0 o2 o3 k1 o4 o5 k2 o6 o7 k3 q0 q1 k4 q2 q3 k5 q4 q5 k6 q6 q7 "
        "g0 b2 g1 b3 g2 g3 g4 g5 g6 g7 g8 g9 g10 g11 g12 g13",
        "y3 f0 y2 f1 o0 o1 o2 o3 y1 o4 o5 o6 o7 y0 f2 x3 f3 x2 q0 q1 q2 q3 x1 q4 q5 q6 q7 W x0 k0 b0 k1 b1 k2 b2 k3 b3 k4 k5 k6 "
        "g0 g1 g2 g3 g4 g5 g6 g7 g8 g9 g10 g11 g12 g13",
    ][POST])
    return " ".join(out)


def timeline(steps):
    load, times = [0] * 4, {}
    for name in steps:
        op, args = name[0], [int(x) for x in name[1:].split('.') if x]
        times[name] = min(load)
        if op in 'KVQO':
            seqs = [DH] * 14 + ([D] * 2 if op in 'QO' else [])
        elif op == 'a':
            seqs = [(args[0] + 1) * T]
        elif op in 'cmvn':
            seqs = [D] * 3 if args[1] == 7 else [DH] * (args[0] if op in 'cm' else NB - 1 - args[0])
        elif op == 'd':
            seqs = [(2 * args[0] + 1) * T] * 2 + [T]
        elif op in 'fb':
            seqs = [CP] * min(4, 15 - 4 * args[0])
        else:
            seqs = {'o': [DH] * 16, 'q': [DH] * 16, 'k': [KH] * 8, 'y': [M] * 4, 'x': [M] * 4, 'g': [KH] * 4}.get(op, [])
        for m in seqs:
            load[load.index(min(load))] += m
    times['end'] = min(load)
    return times


def make_kernel(CH=16, HR=H, IL=16, SK={}, CA=16, PA=64, MARG=250, B0=100, B1=400, HOST=128, LAT=150, WIN=100, ETOK=False, W0=300, W1=300, WR=16, WG=False, XP=4, X0=450, XD=12, XKV=True, PW=800, KR=16, KW=2400, KG=True, PD=100, RC=16):
  STEPS = schedule(**SK).split()
  TIMES = timeline(STEPS)

  def kernel(x_hbm, c_hbm, g_hbm, wq_ref, wuk_ref, wuv_ref, wo_hbm, wr_ref, wg_hbm, wu_hbm, wd_hbm,
             out_hbm, dx_hbm, dc_hbm, dwq_hbm, dwuk_hbm, dwuv_hbm, dwo_hbm, dwr_ref, dwg_hbm, dwu_hbm, dwd_hbm,
             xT_s, xnT_s, gT_s, c_s, bx_s, bg_s, bc_s, xr_s, gr_s, stat_s, r_s, outT_a, dxnT_a, gc_a,
             wq_s, wkv_s, wn_s, dwq_s, dwk_s, dwv_s,
             aq_s, ao_s, akv_s, aqr_s, aor_s, akvT_s, nq_s, no_s, nkv_s, ak_s, cq_s, av_s, cdo_s,
             qT_s, k_s, kT_s, v_s, vT_s, ctxT_s, dqT_s, dob_s,
             z_s, s0_s, s1_s, s2_s, s3_s, p_s, psb_s, dsb_s, dsd_s,
             oh_s, xs_s, dy_s, xsT_s, wrb_s, rs_s, y_a, dxs_a, lb_s, act_s, wT_s, ho_s, hq_s, hkv_s, dn_s, sel_a, key_s, ohf_s,
             hin, hout, stq, stk, stv, xin, xout,
             sem_x, sem_c, sem_g, sem_wo, sem_hin, sem_hout, sem_xin, sem_xout):
    g = pl.program_id(0)
    s_s = (s0_s, s1_s, s2_s, s3_s)

    def blk(i):
        return pl.ds(pl.multiple_of(i * TB, TB), TB)

    def tl(i):
        return pl.ds(pl.multiple_of(i * T, T), T)

    def cp_x(i):
        return pltpu.make_async_copy(x_hbm.at[:, blk(i)], xT_s.at[:, blk(i)], sem_x.at[i])

    def cp_g(i):
        return pltpu.make_async_copy(g_hbm.at[:, blk(i)], gT_s.at[:, blk(i)], sem_g.at[i])

    def cp_c(i):
        return pltpu.make_async_copy(c_hbm.at[blk(i), :], c_s.at[blk(i), :], sem_c.at[i])

    def cp_out(i):
        return pltpu.make_async_copy(xT_s.at[:, blk(i)], out_hbm.at[:, blk(i)], sem_x.at[i])

    def cp_dx(i):
        return pltpu.make_async_copy(gT_s.at[:, blk(i)], dx_hbm.at[:, blk(i)], sem_g.at[i])

    def cp_dc(i):
        return pltpu.make_async_copy(c_s.at[blk(i), :], dc_hbm.at[blk(i), :], sem_c.at[i])

    cp_wo0 = pltpu.make_async_copy(wo_hbm.at[0], hin.at[1, 3], sem_wo.at[0])

    def cps_hin(h, slot):
        hn = jnp.minimum(h + 1, H - 1)
        srcs = [wg_hbm.at[:, tl(h)], wu_hbm.at[:, tl(h)], wd_hbm.at[:, tl(h)], wo_hbm.at[hn]]
        return [pltpu.make_async_copy(s, hin.at[slot, i], sem_hin.at[slot]) for i, s in enumerate(srcs)]

    def cps_hout(h, slot):
        dsts = [dwo_hbm.at[h], dwg_hbm.at[:, tl(h)], dwu_hbm.at[:, tl(h)], dwd_hbm.at[:, tl(h)]]
        cps = [pltpu.make_async_copy(hout.at[slot, i], d, sem_hout.at[0]) for i, d in enumerate(dsts)]
        pair = h // 2
        cps += [pltpu.make_async_copy(s.at[slot], d.at[:, pair], sem_hout.at[0])
                for s, d in ((stq, dwq_hbm), (stk, dwuk_hbm), (stv, dwuv_hbm))]
        return cps

    xcol = pl.ds(H * T, FX)
    cps_xin = [pltpu.make_async_copy(w.at[:, xcol], xin.at[i], sem_xin.at[0]) for i, w in enumerate((wg_hbm, wu_hbm, wd_hbm))]
    cps_xout = [pltpu.make_async_copy(xout.at[i], w.at[:, xcol], sem_xout.at[0]) for i, w in enumerate((dwg_hbm, dwu_hbm, dwd_hbm))]

    def ffn_fwd(wg, wu, wd):
        return ffn_act(dot(xs_s[...], wg), dot(xs_s[...], wu), dot(dy_s[...], wd))

    def ffn_act(a, u, dh):
        rs = rs_s[:, 0:1]
        sg = jax.nn.sigmoid(a)
        gl = a * sg
        dh = dh * rs
        return dh * u * (sg * (1.0 + a * (1.0 - sg))), dh * gl, gl * u * rs

    def ffn_bwd(wg, wu, wd, da, du, hb):
        y_a[...] += dot(hb, wd, NT)
        dxs_a[...] += dot(da, wg, NT) + dot(du, wu, NT)

    def ffn_dw(da, du, hb):
        zero = jnp.zeros(da.shape, bf16)
        q = M // 4
        outs = []
        for rhs in (jnp.concatenate([da, zero], axis=0), jnp.concatenate([du, zero], axis=0), jnp.concatenate([zero, hb], axis=0)):
            outs.append(jnp.concatenate([dot(xsT_s[i * q:(i + 1) * q, 0:2 * CP], rhs).astype(bf16) for i in range(4)], axis=0))
        return outs

    def store_bsums(dst, top, bot, r0, i):
        n = top.shape[0]
        tf, bf_ = top.astype(f32), bot.astype(f32)
        s = sum_b(tf[:, 0:T], tf[:, T:TB], bf_[:, 0:T], bf_[:, T:TB])
        s02, s35 = pk(jnp.concatenate([s[0], s[2]], axis=1)), pk(jnp.concatenate([s[3], s[5]], axis=1))
        vals = [s02[:, 0:T], pltpu.bitcast(top[:, 0:T], u32), s02[:, T:TB], s35[:, 0:T], pltpu.bitcast(bot[:, T:TB], u32),
                s35[:, T:TB], pk(s[6])]
        for r in range(7):
            dst[r, r0 // 2:(r0 + n) // 2, tl(i)] = vals[r]

    def prep_w(n, hn, nslot, wo):
        w = (lambda: wkv_s[0, :, tl(hn % HG)], lambda: wkv_s[1, :, tl(hn % HG)], lambda: wq_s[:, tl(hn % HG)], wo)[n]()
        if n >= 2:
            wn_s[nslot, n - 2] = pltpu.bitcast(w, u32)
        return w

    def prep_rem(n, wT):
        if n >= 2:
            (aqr_s, aor_s)[n - 2][...] = wT[:, 2 * KH:M]

    def prep_sums(n, u, r0, nr, c0, nc, gate=lambda x: x):
        dst, o = ((akv_s, 0), (akv_s, DH // 2), (aq_s, 0), (ao_s, 0))[n]
        q = [gate(u[i * DH // 2 + r0:i * DH // 2 + r0 + nr, j * KH + c0:j * KH + c0 + nc]) for i in range(2) for j in range(2)]
        a = sum_a(*[upk(x).astype(f32) for x in q])
        for r in range(7):
            dst[r, o + r0:o + r0 + nr, c0:c0 + nc] = q[0] if r == 2 else q[3] if r == 3 else pk(a[r])

    @pl.when(g == 0)
    def _():
        cp_wo0.start()
        for cp_ in (cp_x, cp_g, cp_c):

            def start(i, carry):
                cp_(i).start()
                return carry

            lax.fori_loop(0, NB, start, 0)
        for cp in cps_hin(0, 0):
            cp.start()

    @pl.when(g != 1)
    def _():
        wq_s[...] = wq_ref[...].reshape(M, HG * D)
        wkv_s[0] = wuk_ref[...].reshape(DC, HG * D)
        wkv_s[1] = wuv_ref[...].reshape(DC, HG * D)

    @pl.when(g == 0)
    def _():
        cp_wo0.wait()
        z_s[0] = 0
        dwq_s[...] = jnp.zeros(dwq_s.shape, bf16)
        dwk_s[...] = jnp.zeros(dwk_s.shape, bf16)
        dwv_s[...] = jnp.zeros(dwv_s.shape, bf16)
        y_a[...] = jnp.zeros((CP, M), f32)
        dxs_a[...] = jnp.zeros((CP, M), f32)
        wrb_s[...] = jnp.broadcast_to(wr_ref[...].reshape(1, M), (T, M)).T.astype(f32)
        sel_a[...] = jnp.zeros((M, T), f32)
        for n in range(4):
            wT = prep_w(n, 0, 0, lambda: hin[1, 3]).T
            prep_rem(n, wT)
            prep_sums(n, pltpu.bitcast(wT[:, 0:2 * KH], u32), 0, DH // 2, 0, KH)

        def stat_body(i, carry):
            cols = blk(i)
            cp_x(i).wait()
            gc_a[:, :, tl(i)] = jnp.zeros((7, KH, T), f32)
            shift = xT_s[0:16, cols].astype(f32)[0:1, :]
            s1 = s2 = None
            for r0 in range(0, M, RC):
                d = (xT_s[r0:r0 + RC, cols].astype(f32) - shift).reshape(RC // 8, 8, TB)
                a1, a2 = jnp.sum(d, axis=0), jnp.sum(d * d, axis=0)
                s1, s2 = (a1, a2) if s1 is None else (s1 + a1, s2 + a2)
            m1 = jnp.sum(s1, axis=0, keepdims=True) * (1.0 / M)
            var = jnp.maximum(jnp.sum(s2, axis=0, keepdims=True) * (1.0 / M) - m1 * m1, 0.0)
            stat_s[0, :, cols] = rb(shift + m1)
            stat_s[1, :, cols] = 1.0 / rb(jnp.sqrt(rb(rb(var) + EPS_BF16)))
            stat_s[2, :, cols] = lax.rsqrt(var + EPS)
            return carry

        lax.fori_loop(0, NB, stat_body, 0)

        def norm_body(i, carry):
            cols = blk(i)
            cp_g(i).wait()
            mean, inv = stat_s[0, :, cols], stat_s[1, :, cols]
            racc = None

            def rows_(r0):
                xf = xT_s[r0:r0 + RC, cols].astype(f32)
                xn = (rb(xf - mean) * inv).astype(bf16)
                xnT_s[r0:r0 + RC, cols] = xn
                xnf = xn.astype(f32)
                outT_a[r0:r0 + RC, cols] = xf + xnf
                gb = gT_s[r0:r0 + RC, cols]
                dxnT_a[r0:r0 + RC, cols] = gb.astype(f32)
                w = wrb_s[r0:r0 + RC, :]
                return xn, gb, jnp.sum((xnf * jnp.concatenate([w, w], axis=1)).reshape(RC // 8, 8, TB), axis=0)

            for r0 in range(0, KH, RC):
                (xt, gt, p1), (xb, gb, p2) = rows_(r0), rows_(KH + r0)
                store_bsums(bx_s, xt, xb, r0, i)
                store_bsums(bg_s, gt, gb, r0, i)
                racc = p1 + p2 if racc is None else racc + p1 + p2
            for r0 in range(0, MR, RC):
                xn, gb, p = rows_(2 * KH + r0)
                xr_s[r0 // 2:(r0 + RC) // 2, cols] = pltpu.bitcast(xn, u32)
                gr_s[r0 // 2:(r0 + RC) // 2, cols] = pltpu.bitcast(gb, u32)
                racc = racc + p
            r_s[:, cols] = jnp.sum(racc, axis=0, keepdims=True)
            return carry

        lax.fori_loop(0, NB, norm_body, 0)

        r = jnp.broadcast_to(rb(r_s[...]), (C, S))
        bits = pltpu.bitcast(r, jnp.int32)
        code = jnp.where(bits >= 0, bits, -(bits & 0x7FFFFFFF)) >> 16
        pos = lax.broadcasted_iota(jnp.int32, (C, S), 1)
        key_s[...] = pltpu.bitcast(((code + 0x8000) << 11) + (0x20000000 + S - 1 - pos), f32)
        ohf_s[...] = jnp.zeros((C, S), f32)

        def argmax():
            kmax = jnp.max(key_s[...], axis=1, keepdims=True)
            return S - 1 - (pltpu.bitcast(kmax, jnp.int32)[0, 0] & (S - 1))

        def c_body(i, idx):
            cp_c(i).wait()
            hit = pos == idx
            key_s[...] = jnp.where(hit, 0.0, key_s[...])
            nxt = argmax()
            ohf_s[...] = jnp.where(hit & (lax.broadcasted_iota(jnp.int32, (C, S), 0) == i), 1.0, ohf_s[...])
            pick = (lax.broadcasted_iota(jnp.int32, (T, T), 0) == idx % T).astype(f32).astype(bf16)
            hm = M // 2
            lane = lax.broadcasted_iota(jnp.int32, (hm, T), 1)
            for r0 in (0, hm):
                xc = dot(xnT_s[r0:r0 + hm, tl(idx // T)], pick)
                gc = dot(gT_s[r0:r0 + hm, tl(idx // T)], pick)
                lb_s[i, r0:r0 + hm, :] = xc
                lb_s[C + i, r0:r0 + hm, :] = gc
                sel_a[r0:r0 + hm, :] = jnp.where(lane == i, xc, jnp.where(lane == CP + i, gc, sel_a[r0:r0 + hm, :]))
            cT = c_s[blk(i), :].T
            for r0 in range(0, KH, RC):
                store_bsums(bc_s, cT[r0:r0 + RC], cT[KH + r0:KH + r0 + RC], r0, i)
            return nxt

        lax.fori_loop(0, C, c_body, argmax())
        oh = ohf_s[...]
        rs = jax.nn.sigmoid(jnp.sum(jnp.where(oh > 0.0, rb(r_s[...]), 0.0), axis=1, keepdims=True))
        rs_s[...] = jnp.broadcast_to(jnp.concatenate([rs, rs], axis=0), (CP, T))
        oh_s[...] = jnp.concatenate([oh, oh], axis=0).astype(bf16)
        selT = sel_a[...].astype(bf16)
        xsT_s[...] = selT
        sel = selT.T
        xs_s[...] = sel[0:CP]
        dy_s[...] = sel[CP:2 * CP]
        for cp in cps_xin:
            cp.start()

    @pl.when(g == 2)
    def _():
        for cp in cps_xin:
            cp.wait()

        def body(i, carry):
            cols = blk(i)
            wg, wu, wd = xin[0, :, cols], xin[1, :, cols], xin[2, :, cols]
            da, du, hb = [x.astype(bf16) for x in ffn_fwd(wg, wu, wd)]
            ffn_bwd(wg, wu, wd, da, du, hb)
            xout[0, :, cols], xout[1, :, cols], xout[2, :, cols] = ffn_dw(da, du, hb)
            return carry

        lax.fori_loop(0, FX // TB, body, 0)
        for cp in cps_xout:
            cp.start()

    def head(h, carry):
        slot = h % 2
        hn = jnp.minimum(h + 1, H - 1)
        for cp in cps_hin(h, slot):
            cp.wait()

        @pl.when(h > 1)
        def _():
            for cp in cps_hout(h - 2, slot):
                cp.wait()

        @pl.when(h > 0)
        def _():
            for cp in cps_hout(h - 1, 1 - slot):
                cp.start()

        @pl.when(h < HR - 1)
        def _():
            for cp in cps_hin(h + 1, 1 - slot):
                cp.start()

        zw = [z_s[0]]
        tri = (lax.broadcasted_iota(jnp.int32, (T, T), 0) <= lax.broadcasted_iota(jnp.int32, (T, T), 1))
        tile = lambda j: slice(j * T, (j + 1) * T)
        span = lambda j0, j1: slice(j0 * T, j1 * T)
        rows = lambda r0, r1: slice(r0 // 2, r1 // 2)
        st, pend = {}, []
        always = jnp.full((8, T), zw[0], jnp.int32) == 0

        gates, toks = [], []
        load = [0, 0, 0, 0]

        def pin(u, dummy, g=0, c=0):
            row = u[8 * g:8 * g + 8, :]
            cell = jnp.where(always, row[:, c * T:(c + 1) * T], dummy if dummy.dtype == u32 else pltpu.bitcast(dummy, u32))
            parts = ([row[:, :c * T]] if c else []) + [cell] + ([row[:, (c + 1) * T:]] if (c + 1) * T < u.shape[1] else [])
            row = jnp.concatenate(parts, axis=1)
            parts = ([u[:8 * g]] if g else []) + [row] + ([u[8 * g + 8:]] if 8 * g + 8 < u.shape[0] else [])
            return jnp.concatenate(parts, axis=0)

        def run_tasks(upto):
            pend.sort(key=lambda p: p[0])
            toks = []
            while pend and pend[0][0] <= upto:
                when, fn_ = pend.pop(0)
                tok = fn_()
                if tok is not None:
                    toks.append((when, tok))
            return toks

        def mm(lhs, rhs, dims=NN):
            packed = lhs.dtype == u32
            m = lhs.shape[0] * (2 if packed else 1)
            kt = -(-lhs.shape[1] // T)
            nt = -(-rhs.shape[1 if dims == NN else 0] // T)
            st['start'] = min(load)
            for i in range(kt * nt):
                x = load.index(min(load))
                if i < kt and 16 < m and lhs.shape[1] % T == 0:
                    if m <= HOST:
                        toks.extend(run_tasks(load[x] + m - 16))
                    due = [p for p in toks if p[0] <= load[x] + m - 16]
                    toks[:] = [p for p in toks if p[0] > load[x] + m - 16]
                    for when, tok in due:
                        if not packed:
                            lhs, packed = pltpu.bitcast(lhs, u32), True
                        lhs = pin(lhs, tok, max(0, -(-(when - load[x]) // 16)), i)
                if i < kt:
                    last = load[x] if i == 0 else max(last, load[x])
                load[x] += m
            y = dot(upk(lhs) if packed else lhs, rhs, dims)
            if y.shape[1] >= T:
                gates.extend((last + r + LAT, y, r) for r in range(0, m, 32))
            if st.get('post'):
                run_tasks(min(load))
            return y

        def xpose(x, t0=None):
            y = x.T
            if XP:
                u = pltpu.bitcast(y, u32)
                t0 = (min(load) if t0 is None else t0) + X0
                cells = [(r, c) for c in range(0, u.shape[1] // T * T, T) for r in range(8 * XP - 8, u.shape[0], 8 * XP)]
                toks.extend((t0 + XD * XP * (x_ + 1), u[r:r + 8, c:c + T]) for x_, (r, c) in enumerate(cells))
            return y

        def gated(x, when):
            x = jnp.broadcast_to(x, (8, T))
            ok = [g for g in gates if g[0] <= when - WIN]
            if not ok or not WIN:
                return x
            _, y, r = max(ok, key=lambda g: g[0])
            return jnp.where(always, x, y[r:r + 8, 0:T])

        def strassen_fwd(a_of, b_s, t):
            c11, c12, c21, c22 = comb_c([mm(a_of(r), upk(b_s[r, :, tile(t)])) for r in range(7)])
            return jnp.concatenate([c11, c21], axis=0), jnp.concatenate([c12, c22], axis=0)

        def store7(dst, vals, t, r0=0):
            for r in range(7):
                if dst.dtype == u32:
                    dst[zw[0] + r, t, rows(r0, r0 + DH), :] = pk(vals[r])
                else:
                    dst[r, t, r0:r0 + DH, :] = vals[r].astype(bf16)

        def cat(ref, idx, *lead):
            return jnp.concatenate([ref[lead + (i,)] for i in idx], axis=1)

        def quads(tiles):
            return tiles[0][0:DH], tiles[1][0:DH], tiles[0][DH:D], tiles[1][DH:D]

        def kvproj(which, t):
            dst, dstT, dstA = ((k_s, kT_s, ak_s), (v_s, vT_s, av_s))[which]
            tiles = strassen_fwd(lambda r: akv_s[r, rows(which * DH, (which + 1) * DH), :], bc_s, t)
            for e in range(2):
                j = 2 * t + e
                dstT[j] = tiles[e].astype(bf16)
                dst[zw[0], rows(j * T, (j + 1) * T), :] = pltpu.bitcast(xpose(tiles[e].astype(bf16)) if XKV else tiles[e].astype(bf16).T, u32)
            if t < NB - 1:
                store7(dstA, sum_a(*quads(tiles)), t)

        def qproj(t):
            tiles = strassen_fwd(lambda r: aq_s[r], bx_s, t)
            rem = mm(aqr_s[...], upk(xr_s[:, span(2 * t, 2 * t + 2)]))
            tiles = [(tiles[e] + rem[:, tile(e)]) * (SCALE * LOG2E) for e in range(2)]
            for e in range(2):
                qT_s[2 * t + e] = tiles[e].astype(bf16)
            if t > 0:
                store7(cq_s, sum_c(*quads(tiles)), t)

        def doproj(t):
            tiles = strassen_fwd(lambda r: ao_s[r], bg_s, t)
            rem = mm(aor_s[...], upk(gr_s[:, span(2 * t, 2 * t + 2)]))
            tiles = [tiles[e] + rem[:, tile(e)] for e in range(2)]
            for e in range(2):
                dob_s[2 * t + e] = tiles[e].astype(bf16)
            if t > 0:
                store7(cdo_s, sum_c(*quads(tiles)), t)

        blk0 = lambda t: t * (t - 1) // 2
        prow = lambda j, i: (j * (j + 1) // 2 + i) * T
        ptile = lambda j, i: p_s[prow(j, i):prow(j, i) + T, :]

        def a_(j):
            s = mm(k_s[0, rows(0, (j + 1) * T), :], qT_s[j])
            t0, run = st['start'], {}

            def chunk(r0):
                sc = s[r0:r0 + CA, :]
                if r0 >= j * T:
                    sc = jnp.where(tri[r0 - j * T:r0 - j * T + CA, :], sc, NEG)
                s_s[j % 4][zw[0], r0:r0 + CA, :] = sc
                sc = sc.reshape(CA // 8, 8, T)
                mi = jnp.max(sc, axis=0)
                mn = jnp.maximum(run['m'], mi) if run else mi
                li = jnp.sum(jnp.exp2(sc - mn), axis=0)
                run['l'] = run['l'] * jnp.exp2(run['m'] - mn) + li if run else li
                run['m'] = mn
                if r0 + CA == (j + 1) * T:
                    m = jnp.max(mn, axis=0, keepdims=True)
                    st['lse', j] = m + jnp.log2(jnp.sum(run['l'] * jnp.exp2(mn - m), axis=0, keepdims=True))
                return run['l'] if (r0 + CA) % PA == 0 else None

            for r0 in range(0, (j + 1) * T, CA):
                pend.append((t0 + r0 + CA + MARG, functools.partial(chunk, r0)))
            st['aend', j] = t0 + (j + 1) * T + MARG

        PSUM = {0: 0, 2: 1, 3: 2, 5: 3, 6: 4}

        def e_(t, t0, t1):
            j1, j2 = 2 * t, 2 * t + 1
            total, done = (4 * t + 3) * T, 0

            def chunk(u, c0, when):
                r1, r2 = u * TB + c0, u * TB + T + c0
                lse = {j: gated(st['lse', j], when) for j in (j1, j2)}

                def prob(j, r0):
                    p = jnp.exp2(s_s[j % 4][0, r0:r0 + CH, :].reshape(CH // 8, 8, T) - lse[j]).reshape(CH, T)
                    p_s[prow(j, 0) + r0:prow(j, 0) + r0 + CH, :] = p.astype(bf16)
                    return p

                if u < t:
                    sums = sum_b(prob(j1, r1), prob(j2, r1), prob(j1, r2), prob(j2, r2))
                    for r, slot_ in PSUM.items():
                        o = (blk0(t) + u) * T + c0
                        psb_s[slot_, o:o + CH, :] = sums[r].astype(bf16)
                    tok = sums[5] + sums[6]
                else:
                    tok = prob(j1, r1) + prob(j2, r1) + prob(j2, r2)
                st['edone', t] = st.get(('edone', t), 0) + 1
                if PD and u == t and c0 == T - CH:
                    o = pl.multiple_of(prow(NTL - 1, 0) + zw[0] * 16, 16)
                    toks.append((when + PD, p_s[pl.ds(o, 16), :]))
                    toks.append((when + PD, psb_s[zw[0], blk0(NB - 1) * T:blk0(NB - 1) * T + 16, :]))
                return jnp.sum(tok.reshape(CH // 8, 8, T), axis=0) if ETOK else None

            for u in range(t + 1):
                for c0 in range(0, T, CH):
                    done += (4 if u < t else 3) * CH
                    when = t0 + max(t1 - t0, 0) * done // total
                    pend.append((when, functools.partial(chunk, u, c0, when)))

        def pcomb(r, t, u):
            if r in PSUM:
                return psb_s[PSUM[r], tile(blk0(t) + u), :]
            return ptile(2 * t, 2 * u) if r == 1 else ptile(2 * t + 1, 2 * u + 1)

        pdiag = lambda t, e: ptile(2 * t + min(e, 1), 2 * t + e // 2)
        dscomb = lambda r, t, u: dsb_s[r, tile(blk0(t) + u), :]
        dsdiag = lambda t, e: dsd_s[t, e]

        def over_k(name, t, r, a_s, xT_s, comb, diag):
            if r < 7:
                if t > 0:
                    st[name, r] = mm(cat(a_s, range(t), r), jnp.concatenate([comb(r, t, u) for u in range(t)], axis=0))
                return None
            j1, j2 = 2 * t, 2 * t + 1
            y = [mm(xT_s[j1], diag(t, 0)),
                 mm(cat(xT_s, (j1, j2)), jnp.concatenate([diag(t, 1), diag(t, 2)], axis=0))]
            if t > 0:
                c11, c12, c21, c22 = comb_c([st.pop((name, i)) for i in range(7)])
                y = [y[0] + jnp.concatenate([c11, c21], axis=0), y[1] + jnp.concatenate([c12, c22], axis=0)]
            return y

        def over_q(name, u, r, c_s_, xT, comb, diag):
            if r < 7:
                if u < NB - 1:
                    ts = range(NB - 1, u, -1)
                    st[name, r] = mm(cat(c_s_, ts, r),
                                     jnp.concatenate([comb(r, t, u) for t in ts], axis=1), NT)
                return None
            i1, i2 = 2 * u, 2 * u + 1
            y = [mm(cat(xT, (i1, i2)), jnp.concatenate([diag(u, 0), diag(u, 1)], axis=1), NT),
                 mm(xT[i2], diag(u, 2), NT)]
            if u < NB - 1:
                d11, d12, d21, d22 = comb_a([st.pop((name, i)) for i in range(7)])
                y = [y[0] + jnp.concatenate([d11, d21], axis=0), y[1] + jnp.concatenate([d12, d22], axis=0)]
            return y

        def c_(t, r):
            o = over_k('c', t, r, av_s, vT_s, pcomb, pdiag)
            if o is not None:
                for e in range(2):
                    j = 2 * t + e
                    ctxT_s[j] = o[e].astype(bf16)
                    st['delta', j] = jnp.sum(dob_s[j].astype(f32) * o[e], axis=0, keepdims=True)
                store7(no_s, sum_c(*quads(o)), t)

        def q_(t, r):
            dq = over_k('q', t, r, ak_s, kT_s, dscomb, dsdiag)
            if dq is not None:
                dq = [x * SCALE for x in dq]
                for e in range(2):
                    dqT_s[2 * t + e] = dq[e].astype(bf16)
                st['last'] = dq[0][0:8, :]
                store7(nq_s, sum_c(*quads(dq)), t)

        def v_(u, r):
            dv = over_q('v', u, r, cdo_s, dob_s, pcomb, pdiag)
            if dv is not None:
                store7(nkv_s, sum_c(*quads(dv)), u, DH)

        def k_(u, r):
            dk = over_q('k', u, r, cq_s, qT_s, dscomb, dsdiag)
            if dk is not None:
                dk = [x * LN2 for x in dk]
                st['last'] = dk[0][0:8, :]
                store7(nkv_s, sum_c(*quads(dk)), u)

        def d_(t, half):
            j1, j2 = 2 * t, 2 * t + 1
            cut = (t + 1) // 2
            u0, u1 = ((0, cut), (cut, t), (0, t))[half]
            half = min(half, 1)
            n = u1 - u0
            parts = []
            if n:
                v4 = v_s[0, rows(u0 * TB, u1 * TB), :].reshape(n, 2, T // IL, IL // 2, T)
                parts.append(jnp.stack([v4[:, 0], v4[:, 1]], axis=2).reshape(n * T, T))
            if half == 1:
                parts.append(v_s[0, rows(j1 * T, j2 * T), :])
            if not parts:
                return
            dp = mm(jnp.concatenate(parts, axis=0), cat(dob_s, (j1, j2)))
            if n:
                b = {}
                for e, j in enumerate((j1, j2)):
                    d5 = dp[0:n * TB, tile(e)].reshape(n, T // IL, 2, IL, T)
                    p4 = p_s[prow(j, 2 * u0):prow(j, 2 * u1), :].astype(f32).reshape(n, 2, T, T)
                    for i in range(2):
                        b[i, e] = p4[:, i] * (d5[:, :, i].reshape(n, T, T) - st['delta', j])
                sums = sum_b(b[0, 0], b[0, 1], b[1, 0], b[1, 1])
                for r in range(7):
                    dsb_s[r, (blk0(t) + u0) * T:(blk0(t) + u1) * T, :] = sums[r].reshape(n * T, T).astype(bf16)
            if half == 1:
                for e, j in enumerate((j1, j2)):
                    dsd_s[t, e] = (ptile(j, j1).astype(f32) * (dp[n * TB:, tile(e)] - st['delta', j])).astype(bf16)
                dp = mm(v_s[0, rows(j2 * T, (j2 + 1) * T), :], dob_s[j2])
                dsd_s[t, 2] = (ptile(j2, j2).astype(f32) * (dp - st['delta', j2])).astype(bf16)

        def gate_at(when):
            _, y, r = max([g for g in gates if g[0] <= when], key=lambda g: g[0])
            return y[r:r + 8, 0:T]

        def spread(fn_, jobs, t0, t1):
            for x, job in enumerate(jobs):
                when = t0 + max(t1 - t0, 0) * (x + 1) // len(jobs)
                pend.append((when, functools.partial(fn_, *job, when)))

        def prep(n):
            u = pltpu.bitcast(prep_w(n, hn, 1 - slot, lambda: hin[slot, 3]), u32)
            after = gate_at(min(load))
            wT = xpose(upk(jnp.concatenate([pin(u[r:r + T // 2], after) for r in range(0, u.shape[0], T // 2)], axis=0)))
            prep_rem(n, wT)
            wT_s[zw[0] + n] = pltpu.bitcast(wT[:, 0:2 * KH], u32)

            def job(r0, c0, when):
                after = pltpu.bitcast(gate_at(when - WIN), u32)
                prep_sums(n, wT_s.at[n], r0, 8, c0, T, lambda x: jnp.where(always, x, after))

            t0 = min(load) + X0 + 32 * XD + 100
            spread(job, [(r0, c0) for r0 in range(0, DH // 2, 8) for c0 in (0, T)], t0, t0 + PW)

        def stage(st_ref, prev_ref, r0, cur):
            n = cur.shape[0]
            st_ref.at[slot, r0:r0 + n][...] = jnp.concatenate([prev_ref[r0:r0 + n, :], cur], axis=1).reshape(n, 2, D)
            prev_ref[r0:r0 + n, :] = cur

        def dw_top(h_s):
            d11, d12, d21, d22 = comb_a([h_s[r] for r in range(7)])
            top = jnp.concatenate([jnp.concatenate([d11, d12], axis=1), jnp.concatenate([d21, d22], axis=1)], axis=0)
            return xpose(top.astype(bf16))

        def kv_fin(r0, when):
            after = gate_at(when - WIN)
            hs = [hkv_s[r, r0:r0 + KR, :] for r in range(7)]
            for r in (0, 4, 5) if KG else ():
                hs[r] = jnp.where(always, hs[r].reshape(KR // 8, 8, T), after).reshape(KR, T)
            d11, d12, d21, d22 = comb_a(hs)
            lo = lax.broadcasted_iota(jnp.int32, (KR, D), 1) < DH
            for o, da_, db_ in ((0, d11, d21), (KH, d12, d22)):
                sw = pltpu.roll(jnp.where(lo, db_, da_), DH, 1)
                stage(stk, dwk_s, o + r0, jnp.where(lo, da_, sw).astype(bf16))
                stage(stv, dwv_s, o + r0, jnp.where(lo, sw, db_).astype(bf16))

        ffn = {}
        mt = [slice(m0, min(m0 + T, M)) for m0 in range(0, M, T)]
        fwd_q = [(i, m) for i in range(3) for m in mt]
        bwd_q = [(i, m) for m in mt for i in range(3)]

        def step(name):
            op, args = name[0], [int(x) for x in name[1:].split('.') if x]
            n = args[0] if args else 0
            sp = span(4 * n, 4 * n + 4)
            if op == 'K' or op == 'V':
                kvproj('KV'.index(op), n)
            elif op == 'Q':
                qproj(n)
            elif op == 'O':
                doproj(n)
            elif op == 'T':
                for r in range(7):
                    akvT_s[zw[0] + r] = pltpu.bitcast(xpose(upk(akv_s[r]), min(load) + r * 16 * XD), u32)
            elif op == 'a':
                a_(n)
            elif op == 'e':
                e_(n, max(min(load), st['aend', 2 * n], st['aend', 2 * n + 1]) + B0, TIMES['c%d.0' % n] - B1)
            elif op == 'c':
                assert st['edone', n] == (n + 1) * T // CH
                c_(*args)
            elif op == 'v':
                v_(*args)
            elif op == 'd':
                d_(*args)
            elif op == 'm':
                q_(*args)
            elif op == 'n':
                k_(*args)
            elif op == 'o':
                st['post'] = True
                if n < 7:
                    ho_s[zw[0] + n] = mm(cat(no_s, range(NB), n), upk(bg_s[n]), NT)
                else:
                    hout[slot, 0, 2 * KH:M, :] = mm(gr_s[...], cat(ctxT_s, range(NTL)), NT).astype(bf16)
                    hout[slot, 0, 0:2 * KH, :] = dw_top(ho_s)
            elif op == 'q':
                if n < 7:
                    hq_s[zw[0] + n] = mm(cat(nq_s, range(NB), n), upk(bx_s[n]), NT)
                else:
                    stage(stq, dwq_s, 2 * KH, mm(xr_s[...], cat(dqT_s, range(NTL)), NT).astype(bf16))
                    stage(stq, dwq_s, 0, dw_top(hq_s))
            elif op == 'k':
                hkv_s[zw[0] + n] = mm(bc_s[n], cat(nkv_s, range(NB), n), NT)
                if n == 6:
                    spread(kv_fin, [(r0,) for r0 in range(0, KH, KR)], min(load) + 300, min(load) + 300 + KW)
            elif op == 'y':
                outT_a[:, sp] += mm(wn_s[slot, 1], cat(ctxT_s, range(4 * n, 4 * n + 4)))
            elif op == 'x':
                dxnT_a[:, sp] += mm(wn_s[slot, 0], cat(dqT_s, range(4 * n, 4 * n + 4)))
            elif op == 'g':
                r, sp = n // 2, span(4 * (n % 2), 4 * (n % 2) + 4)
                gc_a[r, :, sp] += mm(akvT_s[r], cat(nkv_s, range(4 * (n % 2), 4 * (n % 2) + 4), r))
            elif op == 'f':
                for i, m in fwd_q[4 * n:4 * n + 4]:
                    t = mm((xs_s, xs_s, dy_s)[i][:, m], hin[slot, i, m, :])
                    ffn[i] = t if i not in ffn else ffn[i] + t
            elif op == 'b':
                if 'act' not in ffn:
                    ffn['act'] = ffn_act(ffn[0], ffn[1], ffn[2])
                for i, m in bwd_q[4 * n:4 * n + 4]:
                    (dxs_a, dxs_a, y_a)[i][:, m] += mm(ffn['act'][i].astype(bf16), hin[slot, i, m, :], NT)
            elif op == 'W':
                if 'act' not in ffn:
                    ffn['act'] = ffn_act(ffn[0], ffn[1], ffn[2])
                for i in range(3):
                    act_s[i] = ffn['act'][i][0:C, :]
                t0, t1 = min(load) + W0, TIMES['end'] - W1
                jobs = [(i, r0) for i in range(3) for r0 in range(0, M, WR)]

                def outer(i, r0, when):
                    acc = None
                    for c in range(C):
                        rhs = act_s[i, c:c + 1, :]
                        rhs = gated(rhs, when) if c == 0 or WG else jnp.broadcast_to(rhs, (8, T))
                        t = lb_s[(i // 2) * C + c, r0:r0 + WR, :].reshape(WR // 8, 8, T) * rhs
                        acc = t if acc is None else acc + t
                    hout[slot, 1 + i, r0:r0 + WR, :] = acc.reshape(WR, T).astype(bf16)

                spread(outer, jobs, t0, t1)
            elif op == 'p':
                prep(n)

        for name in STEPS:
            assert TIMES[name] == min(load)
            step(name)
        run_tasks(10 ** 9)

        return carry

    lax.fori_loop(jnp.maximum((g - 1) * (HR // NG) - 1, 0), jnp.where(g == NG, HR, g * (HR // NG) - 1), head, 0)

    @pl.when(g == NG)
    def _():
        for cp in cps_hout(HR - 2, 0):
            cp.wait()
        for cp in cps_hout(HR - 1, 1):
            cp.start()
        rs = rs_s[0:C, 0:1]
        y = y_a[0:C, :]
        xs = xs_s[...].astype(f32)[0:C, :]
        dr = jnp.sum(dy_s[...].astype(f32)[0:C, :] * y, axis=1, keepdims=True) * (1.0 - rs)
        dwr_ref[...] = jnp.sum(dr * xs, axis=0, keepdims=True).astype(bf16).reshape(M)
        de = dxs_a[0:C, :] + dr * wr_ref[...].reshape(1, M).astype(f32)
        yh, deh = rb(y), rb(de)
        xsT_s[...] = jnp.concatenate([yh, y - yh, deh, de - deh, jnp.zeros((T - 4 * C, M), f32)], axis=0).astype(bf16).T

        def body(i, carry):
            cols = blk(i)
            oh = oh_s[:, cols]
            zero = jnp.zeros((CP, TB), bf16)
            hm = M // 2
            scat = lambda rhs: jnp.concatenate([dot(xsT_s[r0:r0 + hm, 0:2 * CP], rhs) for r0 in (0, hm)], axis=0)
            de_, y_ = scat(jnp.concatenate([zero, oh], axis=0)), scat(jnp.concatenate([oh, zero], axis=0))
            z = z_s[0]
            s1 = s2 = None
            for r0 in range(0, M, RC):
                dn = dxnT_a[r0:r0 + RC, cols] + de_[r0:r0 + RC]
                dn_s[z, r0:r0 + RC, :] = dn
                t = (dn * xnT_s[r0:r0 + RC, cols].astype(f32)).reshape(RC // 8, 8, TB)
                a1, a2 = jnp.sum(dn.reshape(RC // 8, 8, TB), axis=0), jnp.sum(t, axis=0)
                s1, s2 = (a1, a2) if s1 is None else (s1 + a1, s2 + a2)
            rstd = stat_s[2, :, cols]
            m1 = jnp.sum(s1, axis=0, keepdims=True) * (rstd * (1.0 / M))
            m2 = jnp.sum(s2, axis=0, keepdims=True) * (rstd * (1.0 / M))
            xT_s[:, cols] = (outT_a[:, cols] + y_).astype(bf16)
            b11, b12, b21, b22 = comb_b([gc_a[r, :, tl(i)] for r in range(7)])
            dcT = jnp.concatenate([jnp.concatenate([b11, b12], axis=1), jnp.concatenate([b21, b22], axis=1)], axis=0)
            c_s[cols, :] = dcT.astype(bf16).T
            cols2 = pl.ds(pl.multiple_of((i + z) * TB, TB), TB)
            for r0 in range(0, M, RC):
                xh = xnT_s[r0:r0 + RC, cols2].astype(f32)
                dxT = (gT_s[r0:r0 + RC, cols].astype(f32) - m1) + (dn_s[0, r0:r0 + RC, :] * rstd - xh * m2)
                gT_s[r0:r0 + RC, cols] = dxT.astype(bf16)
            cp_dc(i).start()
            cp_out(i).start()
            cp_dx(i).start()
            return carry

        lax.fori_loop(0, NB, body, 0)
        for cp in cps_hout(HR - 1, 1):
            cp.wait()
        for cp in cps_xout:
            cp.wait()
        for i in range(NB):
            cp_dc(i).wait()
            cp_out(i).wait()
            cp_dx(i).wait()

  return kernel


def build(NOBC=False, XPK=False, **kw):
  kernel = make_kernel(**kw)

  @jax.jit
  def fn(A_x, A_c_kv, A_w_q, A_w_uk, A_w_uv, A_w_o, B_x, B_w_r, B_w_gate, B_w_up, B_w_down, grad_out):
    hbm = pl.BlockSpec(memory_space=pl.ANY)
    grp = lambda n: pl.BlockSpec((n, HG, D), lambda g: (0, jnp.maximum(g - 1, 0), 0))
    vec = pl.BlockSpec((M,), lambda g: (0,))
    in_specs = [hbm, hbm, hbm, grp(M), grp(DC), grp(DC), hbm, vec, hbm, hbm, hbm]
    out_specs = [hbm, hbm, hbm, hbm, hbm, hbm, hbm, vec, hbm, hbm, hbm]
    sds = lambda *s: jax.ShapeDtypeStruct(s, bf16)
    out_shape = [sds(M, S), sds(M, S), sds(S, DC), sds(M, H // 2, 2, D), sds(DC, H // 2, 2, D), sds(DC, H // 2, 2, D),
                 sds(H, M, D), sds(M), sds(M, F), sds(M, F), sds(M, F)]
    V = pltpu.VMEM
    P = lambda *s: V(s[:-2] + (s[-2] // 2, s[-1]), u32)
    B = lambda *s: V(s, bf16)
    X = P if XPK else B
    DMA = pltpu.SemaphoreType.DMA
    SH = S // 2
    scratch = [
        V((M, S), bf16), V((M, S), bf16), V((M, S), bf16), V((S, DC), bf16),
        P(7, KH, SH), P(7, KH, SH), P(7, KH, SH), P(MR, S), P(MR, S), V((3, 1, S), f32), V((1, S), f32),
        V((M, S), f32), V((M, S), f32), V((7, KH, SH), f32),
        V((M, HG * D), bf16), V((2, DC, HG * D), bf16), P(2, 2, M, D),
        V((M, D), bf16), V((DC, D), bf16), V((DC, D), bf16),
        P(7, DH, KH), P(7, DH, KH), P(7, D, KH), V((D, MR), bf16), V((D, MR), bf16), P(7, KH, D),
        B(7, NB, DH, T), B(7, NB, DH, T), B(7, NB, D, T), X(7, NB, DH, T), X(7, NB, DH, T), X(7, NB, DH, T), X(7, NB, DH, T),
        B(NTL, D, T), P(1, S, D), B(NTL, D, T), P(1, S, D), B(NTL, D, T), B(NTL, D, T), B(NTL, D, T), B(NTL, D, T),
        pltpu.SMEM((1,), jnp.int32), V((1, S, T), f32), V((1, S, T), f32), V((1, S, T), f32), V((1, S, T), f32),
        V((136 * T, T), bf16), V((5, 28 * T, T), bf16), V((7, 28 * T, T), bf16), V((NB, 3, T, T), bf16),
        V((CP, S), bf16), V((CP, M), bf16), V((CP, M), bf16), V((M, 128), bf16), V((M, T), f32), V((CP, 128), f32),
        V((CP, M), f32), V((CP, M), f32), V((2 * C, M, T), f32), V((3, C, T), f32),
        P(4, D, 2 * KH), V((7, DH, KH), f32), V((7, DH, KH), f32), V((7, KH, D), f32), V((1, M, TB), f32), V((M, T), f32), V((C, S), f32), V((C, S), f32),
        V((2, 4, M, T), bf16), V((2, 4, M, T), bf16), V((2, M, 2, D), bf16), V((2, DC, 2, D), bf16), V((2, DC, 2, D), bf16),
        V((3, M, FX), bf16), V((3, M, FX), bf16),
        DMA((NB,)), DMA((NB,)), DMA((NB,)), DMA((1,)), DMA((2,)), DMA((1,)), DMA((1,)), DMA((1,)),
    ]
    outs = pl.pallas_call(
        kernel, grid=(NG + 1,), in_specs=in_specs, out_specs=out_specs, out_shape=out_shape, scratch_shapes=scratch,
        compiler_params=pltpu.CompilerParams(dimension_semantics=("arbitrary",), vmem_limit_bytes=120 * 2 ** 20,
                                             disable_bounds_checks=NOBC),
        name="fused_kernel",
    )(A_x.reshape(S, M).T, A_c_kv.reshape(S, DC), grad_out.reshape(S, M).T, A_w_q, A_w_uk, A_w_uv, A_w_o.transpose(0, 2, 1),
      B_w_r, B_w_gate, B_w_up, B_w_down.T)
    out, dx, dc, dwq, dwuk, dwuv, dwo, dwr, dwg, dwu, dwd = outs
    return (out.T.reshape(1, S, M), dx.T.reshape(1, S, M), dc.reshape(1, S, DC), dwq.reshape(M, H, D), dwuk.reshape(DC, H, D),
            dwuv.reshape(DC, H, D), dwo.transpose(0, 2, 1), dwr, dwg, dwu, dwd.T)

  return fn


_fn = build(NOBC=True)


@jax.jit
def pallas_parallel_sum__compressed_kv_cla__moe_arch_mod__prompt_kernel(
    A_x: jax.Array,
    A_c_kv: jax.Array,
    A_w_q: jax.Array,
    A_w_uk: jax.Array,
    A_w_uv: jax.Array,
    A_w_o: jax.Array,
    B_x: jax.Array,
    B_w_r: jax.Array,
    B_w_gate: jax.Array,
    B_w_up: jax.Array,
    B_w_down: jax.Array,
    grad_out: jax.Array,
):
    return _fn(A_x, A_c_kv, A_w_q, A_w_uk, A_w_uv, A_w_o, B_x, B_w_r, B_w_gate, B_w_up, B_w_down, grad_out)
```

```python
import functools

import jax
import jax.numpy as jnp
from jax import lax
import jax.experimental.pallas as pl
import jax.experimental.pallas.tpu as pltpu

f32 = jnp.float32
bf16 = jnp.bfloat16
u32 = jnp.uint32
i32 = jnp.int32
NN = (((1,), (0,)), ((), ()))
NT = (((1,), (1,)), ((), ()))

S, M, DC, H, D, F, C = 2048, 576, 512, 32, 128, 4608, 8
HG = 8
NG = H // HG
T = 128
NTL = S // T
TB = 2 * T
NB = S // TB
KH = 256
MR = M - 2 * KH
DH = D // 2
DQ = D // 4
NQ = S // (4 * T)
MH = M // 2
CP = 16
FX = F - H * T
EPS = 1e-5
EPS_BF16 = 1.0013580322265625e-05
LOG2E = 1.4426950408889634
LN2 = 0.6931471805599453
SCALE = D ** -0.5
NEG = -1e30


def dot(a, b, dims=NN):
    return lax.dot_general(a, b, dims, preferred_element_type=f32)


def rb(x):
    return x.astype(bf16).astype(f32)


def pk(x):
    return pltpu.bitcast(x.astype(bf16), u32)


def upk(u):
    return pltpu.bitcast(u, bf16)


def vcat(*xs):
    return jnp.concatenate(xs, axis=0) if len(xs) > 1 else xs[0]


def hcat(*xs):
    return jnp.concatenate(xs, axis=1) if len(xs) > 1 else xs[0]


def sum_a(a11, a12, a21, a22):
    return [a11 + a22, a21 + a22, a11, a22, a11 + a12, a21 - a11, a12 - a22]


def sum_b(b11, b12, b21, b22):
    return [b11 + b22, b11, b12 - b22, b21 - b11, b22, b11 + b12, b21 + b22]


def sum_c(c11, c12, c21, c22):
    return [c11 + c22, c21 - c22, c12 + c22, c11 + c21, c12 - c11, c22, c11]


def comb_c(m):
    return m[0] + m[3] - m[4] + m[6], m[2] + m[4], m[1] + m[3], m[0] - m[1] + m[2] + m[5]


def comb_a(m):
    return m[0] + m[2] + m[4] - m[5], m[4] + m[6], m[1] + m[5], m[0] + m[1] + m[3] - m[6]


def comb_b(m):
    return m[0] + m[1] - m[3] + m[5], m[2] + m[5], m[3] + m[6], m[0] - m[2] + m[4] + m[6]


def shear(x, s, sign):
    x11, x12, x21, x22 = x
    h = s * x21
    y11, y22 = (x11 + h, x22 - h) if sign > 0 else (x11 - h, x22 + h)
    return y11, (x12 + s * (x22 - y11) if sign > 0 else x12 - s * (x22 - y11)), x21, y22


def shear_t(x, s, sign):
    x11, x12, x21, x22 = x
    h = s * x12
    y11, y22 = (x11 - h, x22 + h) if sign > 0 else (x11 + h, x22 - h)
    return y11, x12, (x21 + s * (y11 - x22) if sign > 0 else x21 - s * (y11 - x22)), y22


hsum_a = lambda x, s=0.5: sum_a(*shear(x, s, 1))
hsum_b = lambda x, s=0.5: sum_b(*shear(x, s, 1))
hsum_c = lambda x, s=0.5: sum_c(*shear_t(x, s, -1))
hcomb_c = lambda m, s=0.5: shear(comb_c(m), s, -1)
hcomb_a = lambda m, s=0.5: shear_t(comb_a(m), s, 1)
hcomb_b = lambda m, s=0.5: shear_t(comb_b(m), s, 1)


def schedule(PT=(9, 9, -1, -2), NF=3, FILL=4, POST=4, AT=1, TT=0, ORD=2):
    seq = lambda op, t, rs: ["%s%d.%d" % (op, t, r) for r in rs] if 0 <= t < NB else []
    mix = lambda a, b: [x for pair in zip(a, b) for x in pair] if a and b else a + b
    fill = [("L0 L1 L2 L3 Q7 Q6 O7 O6", "a15 a14 O5 O4 O3 O2", "e7 a13 a12 Q5 O1 O0 Q4", "Q3 Q2", "Q1 Q0"),
            ("L0 Q7 L1 Q6 L2 O7 L3 O6 O5 Q5 O4", "a15 a14 a13 a12 O3", "e7 O2 O1 O0 Q4 Q3", "Q2", "Q1 Q0"),
            ("L0 Q7 L1 Q6 L2 L3 O7 O6 O5 Q5", "a15 a14 a13 O4 O3", "e7 a12 O2 O1 O0 Q4", "Q3", "Q2 Q1 Q0"),
            ("L0 L1 L2 L3 Q7 Q6 O7 O6", "a15 a14 a13 O5 O4", "e7 a12 Q5 O3 O2 O1 O0", "Q4 Q3", "Q2 Q1 Q0"),
            ("L0 L1 L2 L3 Q7 Q6 O7 O6", "a15 a14 a13 O5 O4", "e7 a12 Q5 O3 O2 O1 O0 Q4", "Q3", "Q2 Q1 Q0"),
            ("L0 L1 L2 L3 Q7 Q6 O7", "a15 a14 a13 O6 O5", "e7 a12 Q5 O4 O3 O2 O1 O0 Q4", "Q3", "Q2 Q1 Q0")][FILL]
    out = [x for w in fill[0].split() for x in ([w] if w[0] != 'L' else ["%s.%d" % (w, r) for r in range(7)])] + list(fill[1:3])
    for t in range(5, -4, -1):
        if t + 1 >= 0:
            out.append("e%d" % (t + 1))
        if t >= 0:
            out.append("a%d a%d" % (2 * t + 1, 2 * t))
        out += seq("c", t + 2, range(8))
        if t == 5:
            out.append(fill[3])
        out += mix(seq("n", t + 3, range(NF)), seq("m", t + 3, range(NF)))
        if t + 2 >= 0:
            out.append("d%d" % (t + 2))
        if t == 5:
            out.append(fill[4])
        nn, mm, vv = seq("n", t + 3, range(NF, 8)), seq("m", t + 3, range(NF, 8)), seq("v", t + 2, range(8))
        out += [vv + mix(nn, mm), mix(nn, mm) + vv, nn + mix(vv[:len(mm)], mm) + vv[len(mm):],
                mix(vv[:2], mm[:2]) + vv[2:] + mix(nn[:1], mm[2:3]) + nn[1:] + mm[3:]][ORD]
        if AT == t:
            out.append("A")
        if TT == t:
            out.append("T")
        out += ["p%d" % n for n in range(4) if PT[n] == t]
    ky = lambda n, pre="": "k%d.0 y%d.0 k%d.1 %s y%d.1" % (n, 7 + n, n, pre, 7 + n)
    oy = "M o0 o1 y0 o2 y1 o3 f0 y2 o4 f1 y3 o5 f2 y4 o6 f3 y5 o7 y6 "
    qg = " N q0 g0 q1 g1 q2 g2 q3 g3 q4 b0 g4 q5 b1 g5 q6 b2 g6 q7 b3 g7 g8 g9 g10 g11 g12 g13"
    out.append([
        oy + " ".join(ky(n, {0: "W"}.get(n, "")) for n in range(7)) + qg,
        oy + " ".join(ky(n, {0: "W", 2: "p0", 4: "p1"}.get(n, "")) for n in range(7)) + qg,
        oy + " ".join(ky(n, {2: "W", 1: "p0", 3: "p1"}.get(n, "")) for n in range(7)) + qg,
        oy + " ".join(ky(n, {5: "W", 1: "p0", 3: "p1"}.get(n, "")) for n in range(7)) + qg,
        "M o0 o1 y0 o2 y1 o3 f0 y2 o4 f1 y3 o5 f2 y4 o6 f3 y5 o7 y6 k0.0 y7 k0.1 W y8 k1.0 y9 k1.1 p0 y10 k2.0 y11 k2.1 y12 k3.0 y13 N k3.1 p1 "
        "g0 k4.0 g1 k4.1 g2 k5.0 g3 k5.1 g4 k6.0 g5 k6.1 g6.0 q0 g6.1 q1 g7.0 q2 g7.1 q3 b0 g8.0 q4 b1 g8.1 q5 b2 g9.0 q6 b3 g9.1 q7 g10 g11 g12 g13",
        "M o0 o1 y0 o2 y1 o3 f0 y2 o4 f1 y3 o5 f2 y4 o6 f3 y5 o7 y6 q0 y7.0 q1 W y7.1 q2 y8.0 q3 y8.1 q4 b0 y9.0 q5 b1 y9.1 q6 b2 y10.0 q7 b3 y10.1 "
        "k0.0 y11 k0.1 p0 y12 k1.0 y13 N k1.1 g0 k2.0 g1.0 k2.1 p1 g1.1 k3.0 g2.0 k3.1 g2.1 k4.0 g3.0 k4.1 g3.1 k5.0 g4.0 k5.1 g4.1 k6.0 g5 k6.1 "
        "g6 g7 g8 g9 g10 g11 g12 g13",
        "M o0 y0.0 o1 y0.1 o2 y1 o3 f0 y2 o4 f1 y3 o5 f2 y4 o6 f3 y5 o7 y6 k0.0 y7 k0.1 y8 k1.0 p0 y9 k1.1 y10 k2.0 y11 k2.1 p1 y12 k3.0 y13 k3.1 W "
        "g0 k4.0 g1 k4.1 N g2 k5.0 g3 k5.1 g4 k6.0 g5 k6.1 g6.0 q0 g6.1 q1 g7.0 q2 g7.1 q3 b0 g8.0 q4 b1 g8.1 q5 b2 g9.0 q6 b3 g9.1 q7 g10 g11 g12 g13",
    ][POST])
    return " ".join(out).split()


def timeline(steps):
    load, times = [0] * 4, {}
    for name in steps:
        op, args = name[0], [int(x) for x in name[1:].split('.') if x]
        times[name] = min(load)
        if op in 'QO':
            seqs = [DH] * 14 + [D] * 2
        elif op == 'L':
            seqs = [DH] * 7
        elif op == 'a':
            seqs = [(args[0] + 1) * T]
        elif op in 'cmvn':
            seqs = [D] * 3 if args[1] == 7 else [DH] * (args[0] if op in 'cm' else NB - 1 - args[0])
        elif op == 'd':
            seqs = [(2 * args[0] + 1) * T] * 2 + [T]
        elif op == 'k':
            seqs = [DH] * (16 if args[1] == 0 else 12)
        elif op in 'yg' and len(args) > 1:
            seqs = [(MH if op == 'y' else KH) // 2] * 4
        elif op in 'fb':
            seqs = [CP] * min(4, 15 - 4 * args[0])
        else:
            seqs = {'o': [DH] * 16, 'q': [DH] * 16, 'k': [DH] * 28, 'y': [MH] * 4, 'g': [KH] * 4}.get(op, [])
        for m in seqs:
            load[load.index(min(load))] += m
    times['end'] = min(load)
    return times


def make_kernel(SK={}, HR=H, RC=16, CA=16, CH=16, PA=64, MARG=250, B0=100, B1=300, EF=100, EN=6, PD=100, LAT=150, WIN=100,
                XP=8, X0=450, XD=12, PW=1200, A0=0, AW=2000, AD=150, NW=3000, K0=300, KW=2400, W0=300, W1=300, WR=16, L0=330, LW=780, T0=0, TW=1500, M0=300, MK=3, M1=200, DL=150, K1=500, XL=150, LE=450):
  steps = schedule(**SK)
  times = timeline(steps)

  def kernel(x_hbm, c_hbm, g_hbm, wq_ref, wuk_ref, wuv_ref, wo_hbm, wr_ref, wg_hbm, wu_hbm, wd_hbm,
             out_hbm, dx_hbm, dc_hbm, dwq_hbm, dwuk_hbm, dwuv_hbm, dwo_hbm, dwr_ref, dwg_hbm, dwu_hbm, dwd_hbm,
             xT_s, xnT_s, gT_s, c_s, bx_s, bg_s, b2_s, xr_s, gr_s, stat_s, r_s, g2_a, gc_a,
             wq_s, wkv_s, wn_s, wc_s, wT_s, aq_s, ao_s, a4_s, aqr_s, aor_s, akvT_s, a2_s,
             qT_s, k_s, kT_s, v_s, vT_s, doT_s, ctxT_s, dqT_s, ak_s, av_s, cq_s, cdo_s, nq_s, no_s, np_s, nkv_s,
             z_s, s0_s, s1_s, s2_s, s3_s, p_s, psb_s, dsb_s, dsd_s,
             ho_s, hq_s, f0_s, f1_s, f2_s, n2_s, dwT_s, dwq_s, dwk_s, dwv_s,
             wrb_s, key_s, ohf_s, oh_s, sel_a, selT_s, xs_s, dy_s, rs_s, lb_s, act_s, y_a, dxs_a, dn_s, cT_s,
             hin, hout, stq, stk, stv, xin, xout,
             sem_x, sem_c, sem_g, sem_wo, sem_hin, sem_hout, sem_xin, sem_xout):
    g = pl.program_id(0)
    s_s = (s0_s, s1_s, s2_s, s3_s)

    def blk(i):
        return pl.ds(pl.multiple_of(i * TB, TB), TB)

    def tl(i):
        return pl.ds(pl.multiple_of(i * T, T), T)

    copy = pltpu.make_async_copy
    cp_x = lambda i: copy(x_hbm.at[:, blk(i)], xT_s.at[:, blk(i)], sem_x.at[i])
    cp_g = lambda i: copy(g_hbm.at[:, blk(i)], gT_s.at[:, blk(i)], sem_g.at[i])
    cp_c = lambda i: copy(c_hbm.at[blk(i), :], c_s.at[blk(i), :], sem_c.at[i])
    cp_out = lambda i: copy(xT_s.at[:, blk(i)], out_hbm.at[:, blk(i)], sem_x.at[i])
    cp_dx = lambda i: copy(gT_s.at[:, blk(i)], dx_hbm.at[:, blk(i)], sem_g.at[i])
    cp_dc = lambda i: copy(c_s.at[blk(i), :], dc_hbm.at[blk(i), :], sem_c.at[i])
    cp_wo0 = copy(wo_hbm.at[0], hin.at[1, 3], sem_wo.at[0])

    def cps_hin(h, slot):
        srcs = [wg_hbm.at[:, tl(h)], wu_hbm.at[:, tl(h)], wd_hbm.at[:, tl(h)], wo_hbm.at[jnp.minimum(h + 1, H - 1)]]
        return [copy(s, hin.at[slot, i], sem_hin.at[0]) for i, s in enumerate(srcs)]

    def cps_hout(h, slot):
        dsts = [dwo_hbm.at[h], dwg_hbm.at[:, tl(h)], dwu_hbm.at[:, tl(h)], dwd_hbm.at[:, tl(h)]]
        return ([copy(hout.at[slot, i], d, sem_hout.at[0]) for i, d in enumerate(dsts)] +
                [copy(s.at[slot], d.at[:, h >> 1], sem_hout.at[0]) for s, d in ((stq, dwq_hbm), (stk, dwuk_hbm), (stv, dwuv_hbm))])

    xcol = pl.ds(H * T, FX)
    cps_xin = [copy(w.at[:, xcol], xin.at[i], sem_xin.at[0]) for i, w in enumerate((wg_hbm, wu_hbm, wd_hbm))]
    cps_xout = [copy(xout.at[i], w.at[:, xcol], sem_xout.at[0]) for i, w in enumerate((dwg_hbm, dwu_hbm, dwd_hbm))]

    def ffn_act(a, u, dh):
        rs = rs_s[:, 0:1]
        sg = jax.nn.sigmoid(a)
        gl = a * sg
        dh = dh * rs
        return dh * u * (sg * (1.0 + a * (1.0 - sg))), dh * gl, gl * u * rs

    def store_bsums(dst, top, bot, r0, i):
        n = top.shape[0]
        tf, bf_ = top.astype(f32), bot.astype(f32)
        s = sum_b(tf[:, 0:T], tf[:, T:TB], bf_[:, 0:T], bf_[:, T:TB])
        s02, s35 = pk(hcat(s[0], s[2])), pk(hcat(s[3], s[5]))
        vals = [s02[:, 0:T], pltpu.bitcast(top[:, 0:T], u32), s02[:, T:TB], s35[:, 0:T], pltpu.bitcast(bot[:, T:TB], u32),
                s35[:, T:TB], pk(s[6])]
        for r in range(7):
            dst[r, i, r0 // 2:(r0 + n) // 2, :] = vals[r]

    def prep_w(n, hn, nslot, wo):
        col = tl(hn & (HG - 1))
        w = (lambda: wkv_s[0, :, col], lambda: wkv_s[1, :, col], lambda: wq_s[:, col], wo)[n]()
        if n >= 2:
            wn_s[nslot, n - 2] = pltpu.bitcast(w, u32)
        else:
            wc_s[n] = pltpu.bitcast(w, u32)
        return w

    def prep_rem(n, wT):
        if n >= 2:
            (aqr_s, aor_s)[n - 2][...] = wT[:, 2 * KH:M]

    def prep_sums(n, u, r0, nr, c0, nc, gate=lambda x: x):
        dst, o = (aq_s, ao_s)[n - 2], 0
        q = [gate(u[i * DH // 2 + r0:i * DH // 2 + r0 + nr, j * KH + c0:j * KH + c0 + nc]) for i in range(2) for j in range(2)]
        a = sum_a(*[upk(x).astype(f32) for x in q])
        for r in range(7):
            dst[r, o + r0:o + r0 + nr, c0:c0 + nc] = q[0] if r == 2 else q[3] if r == 3 else pk(a[r])

    def prep_lvl1(n, u, z, i2, j2, r0, nr, s=0.5):
        q = [upk(u[(2 * i1 + i2) * DQ // 2 + r0 // 2:(2 * i1 + i2) * DQ // 2 + (r0 + nr) // 2, (2 * j1 + j2) * T:(2 * j1 + j2 + 1) * T])
             for i1 in range(2) for j1 in range(2)]
        for r, a in enumerate(hsum_a([x.astype(f32) for x in q], s)):
            f0_s[z + r, 2 * i2 + j2, n * DQ + r0:n * DQ + r0 + nr, :] = a

    def prep_lvl2(n, r, r0, nr, s=0.5):
        for r2, a in enumerate(hsum_a([f0_s[r, x, n * DQ + r0:n * DQ + r0 + nr, :] for x in range(4)], s)):
            a4_s[7 * r + r2, (n * DQ + r0) // 2:(n * DQ + r0 + nr) // 2, :] = pk(a)

    def unpack_window():
        wq_s[...] = wq_ref[...].reshape(M, HG * D)
        wkv_s[0] = wuk_ref[...].reshape(DC, HG * D)
        wkv_s[1] = wuv_ref[...].reshape(DC, HG * D)

    @pl.when(g == 0)
    def _():
        cp_wo0.start()
        for cp_ in (cp_x, cp_g, cp_c):

            def start(i, carry):
                cp_(i).start()
                return carry

            lax.fori_loop(0, NB, start, 0)
        for cp in cps_hin(0, 0):
            cp.start()

    @pl.when(g != 1)
    def _():
        unpack_window()

    @pl.when(g == 0)
    def _():
        cp_wo0.wait()
        z_s[0] = 0
        for ref in (dwq_s, dwk_s, dwv_s, y_a, dxs_a, sel_a, ohf_s):
            ref[...] = jnp.zeros(ref.shape, ref.dtype)
        wn_s[1, 1] = jnp.zeros((MH, D), u32)
        wrb_s[...] = jnp.broadcast_to(wr_ref[...].reshape(1, M), (T, M)).T.astype(f32)
        for n in range(4):
            wT = prep_w(n, 0, 0, lambda: hin[1, 3]).T
            prep_rem(n, wT)
            u = pltpu.bitcast(wT[:, 0:2 * KH], u32)
            if n >= 2:
                prep_sums(n, u, 0, DH // 2, 0, KH)
            else:
                for x in range(4):
                    prep_lvl1(n, u, 0, x // 2, x % 2, 0, DQ)
                for r in range(7):
                    prep_lvl2(n, r, 0, DQ)

        def stat_body(i, carry):
            cols = blk(i)
            cp_x(i).wait()
            np_s[:, i] = jnp.zeros((7, DH // 2, T), u32)
            shift = xT_s[0:16, cols].astype(f32)[0:1, :]
            s1 = s2 = None
            for r0 in range(0, M, 2 * RC):
                d = (xT_s[r0:r0 + 2 * RC, cols].astype(f32) - shift).reshape(RC // 4, 8, TB)
                a1, a2 = jnp.sum(d, axis=0), jnp.sum(d * d, axis=0)
                s1, s2 = (a1, a2) if s1 is None else (s1 + a1, s2 + a2)
            m1 = jnp.sum(s1, axis=0, keepdims=True) * (1.0 / M)
            var = jnp.maximum(jnp.sum(s2, axis=0, keepdims=True) * (1.0 / M) - m1 * m1, 0.0)
            stat_s[0, :, cols] = rb(shift + m1)
            stat_s[1, :, cols] = 1.0 / rb(jnp.sqrt(rb(rb(var) + EPS_BF16)))
            stat_s[2, :, cols] = lax.rsqrt(var + EPS)
            return carry

        lax.fori_loop(0, NB, stat_body, 0)

        def norm_body(i, carry):
            cols = blk(i)
            cp_g(i).wait()
            mean, inv = stat_s[0, :, cols], stat_s[1, :, cols]
            racc = None

            def rows_(r0):
                xn = (rb(xT_s[r0:r0 + RC, cols].astype(f32) - mean) * inv).astype(bf16)
                xnT_s[r0:r0 + RC, cols] = xn
                w = wrb_s[r0:r0 + RC, :]
                return xn, gT_s[r0:r0 + RC, cols], jnp.sum((xn.astype(f32) * hcat(w, w)).reshape(RC // 8, 8, TB), axis=0)

            for r0 in range(0, KH, RC):
                (xt, gt, p1), (xb, gb, p2) = rows_(r0), rows_(KH + r0)
                store_bsums(bx_s, xt, xb, r0, i)
                store_bsums(bg_s, gt, gb, r0, i)
                racc = p1 + p2 if racc is None else racc + p1 + p2
            for r0 in range(0, MR, RC):
                xn, gb, p = rows_(2 * KH + r0)
                xr_s[r0 // 2:(r0 + RC) // 2, cols] = pltpu.bitcast(xn, u32)
                gr_s[r0 // 2:(r0 + RC) // 2, cols] = pltpu.bitcast(gb, u32)
                racc = racc + p
            r_s[:, cols] = jnp.sum(racc, axis=0, keepdims=True)
            return carry

        lax.fori_loop(0, NB, norm_body, 0)

        bits = pltpu.bitcast(jnp.broadcast_to(rb(r_s[...]), (C, S)), i32)
        code = jnp.where(bits >= 0, bits, -(bits & 0x7FFFFFFF)) >> 16
        pos = lax.broadcasted_iota(i32, (C, S), 1)
        key_s[...] = pltpu.bitcast(((code + 0x8000) << 11) + (0x20000000 + S - 1 - pos), f32)

        def argmax():
            kmax = jnp.max(key_s[...], axis=1, keepdims=True)
            return S - 1 - (pltpu.bitcast(kmax, i32)[0, 0] & (S - 1))

        def route(i, idx):
            hit = pos == idx
            key_s[...] = jnp.where(hit, 0.0, key_s[...])
            nxt = argmax()
            ohf_s[...] = jnp.where(hit & (lax.broadcasted_iota(i32, (C, S), 0) == i), 1.0, ohf_s[...])
            pick = (lax.broadcasted_iota(i32, (T, T), 0) == (idx & (T - 1))).astype(f32).astype(bf16)
            lane = lax.broadcasted_iota(i32, (MH, T), 1)
            for r0 in (0, MH):
                xc = dot(xnT_s[r0:r0 + MH, tl(idx >> 7)], pick)
                gc = dot(gT_s[r0:r0 + MH, tl(idx >> 7)], pick)
                lb_s[0, i, r0:r0 + MH, :] = xc
                lb_s[1, i, r0:r0 + MH, :] = gc
                sel_a[r0:r0 + MH, :] = jnp.where(lane == i, xc, jnp.where(lane == CP + i, gc, sel_a[r0:r0 + MH, :]))
            return nxt

        def c_body(i, idx):
            cp_c(2 * i).wait()
            cp_c(2 * i + 1).wait()
            nxt = route(2 * i + 1, route(2 * i, idx))
            cT_s[z_s[0]] = pltpu.bitcast(c_s[pl.ds(pl.multiple_of(i * 4 * T, 4 * T), 4 * T), :].T, u32)
            for r0 in range(0, T, 16):
                blkv = lambda j, l: upk(cT_s[0, (j * T + r0) // 2:(j * T + r0) // 2 + 8, l * T:(l + 1) * T]).astype(f32)
                lvl1 = [hsum_b([blkv(2 * j1 + j2, 2 * l1 + l2) for j1 in range(2) for l2 in range(2)])
                        for j2 in range(2) for l1 in range(2)]
                for r in range(7):
                    b = hsum_b([x[r] for x in lvl1])
                    for r2 in range(0, 7, 2):
                        u = pk(hcat(*b[r2:r2 + 2]))
                        for e in range(u.shape[1] // T):
                            b2_s[7 * r + r2 + e, i, r0 // 2:r0 // 2 + 8, :] = u[:, e * T:(e + 1) * T]
            return nxt

        lax.fori_loop(0, NQ, c_body, argmax())
        oh = ohf_s[...]
        rs = jax.nn.sigmoid(jnp.sum(jnp.where(oh > 0.0, rb(r_s[...]), 0.0), axis=1, keepdims=True))
        rs_s[...] = jnp.broadcast_to(vcat(rs, rs), (CP, T))
        oh_s[...] = vcat(oh, oh).astype(bf16)
        selT = sel_a[...].astype(bf16)
        selT_s[...] = selT
        sel = selT.T
        xs_s[...] = sel[0:CP]
        dy_s[...] = sel[CP:2 * CP]
        for cp in cps_xin:
            cp.start()

    @pl.when(g == 2)
    def _():
        for cp in cps_xin:
            cp.wait()

        def body(i, carry):
            cols = blk(i)
            w = [xin[n, :, cols] for n in range(3)]
            act = [x.astype(bf16) for x in ffn_act(dot(xs_s[...], w[0]), dot(xs_s[...], w[1]), dot(dy_s[...], w[2]))]
            y_a[...] += dot(act[2], w[2], NT)
            dxs_a[...] += dot(act[0], w[0], NT) + dot(act[1], w[1], NT)
            zero = jnp.zeros((CP, TB), bf16)
            for n in range(3):
                rhs = vcat(act[n], zero) if n < 2 else vcat(zero, act[n])
                xout[n, :, cols] = dot(selT_s[:, 0:2 * CP], rhs).astype(bf16)
            return carry

        lax.fori_loop(0, FX // TB, body, 0)
        for cp in cps_xout:
            cp.start()

    def head(h, carry):
        slot = h & 1
        hn = jnp.minimum(h + 1, H - 1)
        for cp in cps_hin(h, slot):
            cp.wait()

        @pl.when(h > 1)
        def _():
            for cp in cps_hout(h - 2, slot):
                cp.wait()

        @pl.when(h > 0)
        def _():
            for cp in cps_hout(h - 1, 1 - slot):
                cp.start()

        @pl.when(h < HR - 1)
        def _():
            for cp in cps_hin(h + 1, 1 - slot):
                cp.start()

        z = z_s[0]
        always = jnp.full((8, T), z, i32) == 0
        lo = lax.broadcasted_iota(i32, (8, T), 1) < DH
        tile = lambda j: slice(j * T, (j + 1) * T)
        rows = lambda r0, r1: slice(r0 // 2, r1 // 2)
        st, ffn = {}, {}
        load = [0, 0, 0, 0]
        tasks = []
        toks = []
        gates = []

        def pin(u, tok, r=0, c=0):
            row = u[8 * r:8 * r + 8, :]
            cell = lax.select(always, row[:, tile(c)], tok if tok.dtype == u32 else pltpu.bitcast(tok, u32))
            row = hcat(*([row[:, :c * T]] if c else []), cell, *([row[:, (c + 1) * T:]] if (c + 1) * T < u.shape[1] else []))
            return vcat(*([u[:8 * r]] if r else []), row, *([u[8 * r + 8:]] if 8 * r + 8 < u.shape[0] else []))

        def gate(when):
            _, y, r = max([x for x in gates if x[0] <= when], key=lambda x: x[0])
            return y[r:r + 8, 0:T]

        def run_tasks(upto):
            tasks.sort(key=lambda x: x[0])
            while tasks and tasks[0][0] <= upto:
                tasks.pop(0)[2]()
                tasks.sort(key=lambda x: x[0])

        def spread(name, fn, jobs, t0, t1):
            for x, job in enumerate(jobs):
                when = t0 + (t1 - t0) * (x + 1) // len(jobs)
                tasks.append((when, name, functools.partial(fn, *job, when)))

        def due(when, x):
            if DL:
                toks.append((when + DL, x[0:8]))

        def done(name):
            return not any(x[1] == name for x in tasks)

        def mm(lhs, rhs, dims=NN):
            packed = lhs.dtype == u32
            m = lhs.shape[0] * (2 if packed else 1)
            kt = -(-lhs.shape[1] // T)
            nt = -(-rhs.shape[1 if dims == NN else 0] // T)
            st['start'] = last = min(load)
            for i in range(kt * nt):
                x = load.index(min(load))
                if i < kt:
                    last = max(last, load[x])
                    if m > 16 and lhs.shape[1] % T == 0:
                        for when, tok in [p for p in toks if p[0] <= load[x] + m - 16]:
                            if not packed:
                                lhs, packed = pltpu.bitcast(lhs, u32), True
                            lhs = pin(lhs, tok, max(0, -(-(when - load[x]) // 16)), i)
                        toks[:] = [p for p in toks if p[0] > load[x] + m - 16]
                load[x] += m
            y = dot(upk(lhs) if packed else lhs, rhs, dims)
            if y.shape[1] >= T:
                gates.extend((last + r + LAT, y, r) for r in range(0, m, 32))
            run_tasks(min(load))
            return y

        def mmi(lhs, rhs, dims=NN):
            n = DH // 16
            y = mm(vcat(*[lhs[16 * r:16 * r + 16] for i in range(n) for r in (i, n + i)]), rhs, dims).reshape(n, 2, 16, T)
            return y[:, 0].reshape(DH, T), y[:, 1].reshape(DH, T)

        def xpose(x, t0=0):
            y = x.T
            u = pltpu.bitcast(y, u32)
            cells = [(r, c) for c in range(u.shape[1] // T) for r in range(8 * XP - 8, u.shape[0], 8 * XP)]
            toks.extend((min(load) + t0 + X0 + XD * XP * (i + 1), u[r:r + 8, tile(c)]) for i, (r, c) in enumerate(cells))
            return y

        def cat(ref, idx, *lead):
            return hcat(*[ref[lead + (i,)] for i in idx])

        def store7(dst, vals, t, r0=0):
            for r in range(7):
                dst[r, t, r0:r0 + DH, :] = vals[r].astype(bf16)

        def store2(dst, t, q):
            dst[2 * t] = vcat(q[0], q[2]).astype(bf16)
            dst[2 * t + 1] = vcat(q[1], q[3]).astype(bf16)

        def proj(a_of, b_s, t, rem=None):
            q = comb_c([mm(a_of(r), upk(b_s[r, t])) for r in range(7)])
            if rem is not None:
                y = mm(rem[0][...], upk(rem[1][:, t * TB:(t + 1) * TB]))
                q = [q[2 * i + j] + y[i * DH:(i + 1) * DH, tile(j)] for i in range(2) for j in range(2)]
            return q

        def half(when):
            s = lax.select(always, jnp.full((8, T), 0.5, f32), gate(when - WIN))
            return vcat(s, s)

        def gated(xs, idx, when):
            after = gate(when - WIN)
            return [lax.select(vcat(always, always), x, vcat(after, after)) if i in idx else x for i, x in enumerate(xs)]

        def xpose_at(x, when):
            return xpose(upk(pin(pltpu.bitcast(x, u32), gate(when - WIN))))

        def latent(b, r):
            f_s = (f0_s, f1_s, f2_s)[b % 3]
            assert done('L%d' % (b - 3))
            for x, y in enumerate(hcomb_c([mm(a4_s[7 * r + r2], upk(b2_s[7 * r + r2, b])) for r2 in range(7)])):
                f_s[z + r, x] = y
            if r < 6:
                return

            def job(which, l1, i2, r0, when):
                dst, dstT, dstA = ((k_s, kT_s, ak_s), (v_s, vT_s, av_s))[which]
                t, o = 2 * b + l1, i2 * DQ + r0
                q = hcomb_c(gated([f_s[i, 2 * i2 + l1, which * DQ + r0:which * DQ + r0 + 16, :] for i in range(7)], (0, 1, 4), when))
                for x in range(4):
                    dstT[2 * t + x % 2, (x // 2) * DH + o:(x // 2) * DH + o + 16, :] = q[x].astype(bf16)
                if t < NB - 1:
                    for i, a in enumerate(sum_a(*q)):
                        dstA[i, t, o:o + 16, :] = a.astype(bf16)
                if o == DH - 16:
                    def flip():
                        for j in (2 * t, 2 * t + 1):
                            dst[z, rows(j * T, (j + 1) * T), :] = pltpu.bitcast(xpose_at(dstT[j], when + XL), u32)

                    tasks.append((when + XL, 'X', flip))

            spread('L%d' % b, job, [(w, l1, i2, r0) for w in range(2) for l1 in range(2) for i2 in range(2) for r0 in (0, 16)],
                   min(load) + L0, min(load) + L0 + (LW if b < NQ - 1 else LE))

        def qproj(t):
            q = [x * (SCALE * LOG2E) for x in proj(lambda r: aq_s[r], bx_s, t, (aqr_s, xr_s))]
            store2(qT_s, t, q)
            if t > 0:
                store7(cq_s, sum_c(*q), t)

        def doproj(t):
            q = proj(lambda r: ao_s[r], bg_s, t, (aor_s, gr_s))
            store2(doT_s, t, q)
            if t > 0:
                store7(cdo_s, sum_c(*q), t)

        blk0 = lambda t: t * (t - 1) // 2
        pidx = lambda j, i: j * (j + 1) // 2 + i
        PSUM = {0: 0, 2: 1, 3: 2, 5: 3, 6: 4}

        def a_(j):
            assert done('e%d' % (j // 2 + 2)) and done('L%d' % (NQ - 1)) and done('X')
            s = mm(k_s[0, rows(0, (j + 1) * T), :], qT_s[j])
            t0, n, mx, l = st['start'], T // CA, None, None
            for i in range(j + 1):
                si = s[tile(i), :]
                if i == j:
                    si = jnp.where(lax.broadcasted_iota(i32, (T, T), 0) <= lax.broadcasted_iota(i32, (T, T), 1), si, NEG)
                s_s[j % 4][z, i] = si
                si = si.reshape(n, CA // 8, 8, T)
                mi = jnp.max(si, axis=1)
                run = [mx]
                for u in range(n):
                    run.append(mi[u:u + 1] if run[-1] is None else jnp.maximum(run[-1], mi[u:u + 1]))
                mn = vcat(*run[1:])
                li = jnp.sum(jnp.exp2(si - mn[:, None]), axis=1)
                u0 = 0 if i else 1
                alpha = jnp.exp2(vcat(*run[u0:n]) - mn[u0:])
                for u in range(n):
                    l = li[0:1] if l is None else l * alpha[u - u0:u - u0 + 1] + li[u:u + 1]
                    if ((u + 1) * CA) % PA == 0:
                        toks.append((t0 + i * T + (u + 1) * CA + MARG, l[0]))
                mx = run[-1]
            m = jnp.max(mx[0], axis=0, keepdims=True)
            st['lse', j] = jnp.broadcast_to(m + jnp.log2(jnp.sum(l[0] * jnp.exp2(mx[0] - m), axis=0, keepdims=True)), (8, T))
            st['aend', j] = t0 + (j + 1) * T + MARG

        def e_(t, t0, t1):
            j1, j2, n = 2 * t, 2 * t + 1, T // CH
            at = lambda x: t0 + (t1 - t0) * x // ((4 * t + 3) * n)

            def block(u):
                after = [gate(at(4 * u * n + (4 if u < t else 3) * (c + 1)) - WIN) for c in range(n)]
                p = {}
                for j, w in ((j1, 2 if u < t else 1), (j2, 2)):
                    lse = vcat(*[lax.select(always, st['lse', j], x) for x in after]).reshape(1, n, 1, 8, T)
                    p[j] = jnp.exp2(s_s[j % 4][0, 2 * u:2 * u + w].reshape(w, n, CH // 8, 8, T) - lse).reshape(w, T, T)
                    p_s[pidx(j, 2 * u):pidx(j, 2 * u) + w] = p[j].astype(bf16)
                if u < t:
                    sums = sum_b(p[j1][0], p[j2][0], p[j1][1], p[j2][1])
                    for r, x in PSUM.items():
                        psb_s[x, blk0(t) + u] = sums[r].astype(bf16)
                else:
                    toks.append((t1 + PD, p_s[z + pidx(NTL - 1, 0), 0:16, :]))
                    toks.append((t1 + PD, psb_s[z, blk0(NB - 1), 0:16, :]))

            for u in range(t + 1):
                tasks.append((at(min(4 * u + 4, 4 * t + 3) * n) - WIN, 'e%d' % t, functools.partial(block, u)))

        def pcomb(r, t, u):
            return psb_s[PSUM[r], blk0(t) + u] if r in PSUM else p_s[pidx(2 * t, 2 * u) if r == 1 else pidx(2 * t + 1, 2 * u + 1)]

        def pcol(r, t):
            if r in PSUM:
                return psb_s[PSUM[r], blk0(t):blk0(t) + t].reshape(t * T, T)
            return vcat(*[pcomb(r, t, u) for u in range(t)])

        pdiag = lambda t, e: p_s[pidx(2 * t + min(e, 1), 2 * t + e // 2)]
        dscomb = lambda r, t, u: dsb_s[r, blk0(t) + u]
        dscol = lambda r, t: dsb_s[r, blk0(t):blk0(t) + t].reshape(t * T, T)
        dsdiag = lambda t, e: dsd_s[t, e]

        def over_k(name, t, r, a_s, xT_s_, col, diag):
            if r < 7:
                if t > 0:
                    st[name, r] = mm(cat(a_s, range(t), r), col(r, t))
                return None
            (y11, y21), (y12, y22) = mmi(xT_s_[2 * t], diag(t, 0)), mmi(cat(xT_s_, (2 * t, 2 * t + 1)), vcat(diag(t, 1), diag(t, 2)))
            y = [y11, y12, y21, y22]
            return [a + b for a, b in zip(y, comb_c([st.pop((name, i)) for i in range(7)]))] if t > 0 else y

        def over_q(name, u, r, c_s_, xT_s_, comb, diag):
            if r < 7:
                if u < NB - 1:
                    ts = range(NB - 1, u, -1)
                    st[name, r] = mm(cat(c_s_, ts, r), hcat(*[comb(r, t, u) for t in ts]), NT)
                return None
            (y11, y21), (y12, y22) = (mmi(cat(xT_s_, (2 * u, 2 * u + 1)), hcat(diag(u, 0), diag(u, 1)), NT),
                                      mmi(xT_s_[2 * u + 1], diag(u, 2), NT))
            y = [y11, y12, y21, y22]
            return [a + b for a, b in zip(y, comb_a([st.pop((name, i)) for i in range(7)]))] if u < NB - 1 else y

        def c_(t, r):
            o = over_k('c', t, r, av_s, vT_s, pcol, pdiag)
            if o is not None:
                store2(ctxT_s, t, o)
                for e in range(2):
                    st['delta', 2 * t + e] = jnp.sum(doT_s[2 * t + e].astype(f32) * vcat(o[e], o[2 + e]), axis=0, keepdims=True)
                store7(no_s, sum_c(*o), t)

        def m_(t, r):
            dq = over_k('m', t, r, ak_s, kT_s, dscol, dsdiag)
            if dq is not None:
                dq = [x * SCALE for x in dq]
                store2(dqT_s, t, dq)
                store7(nq_s, sum_c(*dq), t)

        def v_(u, r):
            dv = over_q('v', u, r, cdo_s, doT_s, pcomb, pdiag)
            if dv is not None:
                store7(nkv_s, hsum_c(dv), u, DH)

        def n_(u, r):
            dk = over_q('n', u, r, cq_s, qT_s, dscomb, dsdiag)
            if dk is not None:
                store7(nkv_s, hsum_c([x * LN2 for x in dk]), u)

        def dkv2(r, b, which, r0, when):
            o = which * DH + r0
            x = [nkv_s[r, 2 * b + l1, o + i2 * DQ:o + i2 * DQ + 16, :].astype(f32) for i2 in range(2) for l1 in range(2)]
            n = hsum_c(x, half(when))
            for r2 in range(7):
                n2_s[7 * r + r2, b, which * DQ + r0:which * DQ + r0 + 16, :] = n[r2].astype(bf16)
            due(when, n[0])

        def d_(t):
            j1, j2 = 2 * t, 2 * t + 1
            lhs = v_s[0, rows(j1 * T, j2 * T), :]
            if t:
                v4 = v_s[0, rows(0, t * TB), :].reshape(t, 2, T // 16, 8, T)
                lhs = vcat(jnp.stack([v4[:, 0], v4[:, 1]], axis=2).reshape(t * T, T), lhs)
            dp = mm(lhs, cat(doT_s, (j1, j2)))
            if t:
                b = {}
                for e, j in enumerate((j1, j2)):
                    d5 = dp[0:t * TB, tile(e)].reshape(t, T // 16, 2, 16, T)
                    p4 = p_s[pidx(j, 0):pidx(j, j1)].astype(f32).reshape(t, 2, T, T)
                    for i in range(2):
                        b[i, e] = p4[:, i] * (d5[:, :, i].reshape(t, T, T) - st['delta', j])
                sums = sum_b(b[0, 0], b[0, 1], b[1, 0], b[1, 1])
                for r in range(7):
                    dsb_s[r, blk0(t):blk0(t) + t] = sums[r].astype(bf16)
            for e, j in enumerate((j1, j2)):
                dsd_s[t, e] = (pdiag(t, e).astype(f32) * (dp[t * TB:, tile(e)] - st['delta', j])).astype(bf16)
            dp = mm(v_s[0, rows(j2 * T, (j2 + 1) * T), :], doT_s[j2])
            dsd_s[t, 2] = (pdiag(t, 2).astype(f32) * (dp - st['delta', j2])).astype(bf16)

        def prep(n):
            assert done('A') and done('T')
            u = pltpu.bitcast(prep_w(n, hn, 1 - slot, lambda: hin[slot, 3]), u32)
            after = gate(min(load))
            wT = xpose(upk(vcat(*[pin(u[r:r + T // 2], after) for r in range(0, u.shape[0], T // 2)])))
            prep_rem(n, wT)
            wT_s[z + n] = pltpu.bitcast(wT[:, 0:2 * KH], u32)

            def job(r0, c0, when):
                after = pltpu.bitcast(gate(when - WIN), u32)
                prep_sums(n, wT_s.at[n], r0, 8, c0, T, lambda x: lax.select(always, x, after))

            def job2(lvl, x, r0, when):
                if lvl == 1:
                    prep_lvl1(n, wT_s.at[n], z, x // 2, x % 2, r0, 16, half(when))
                else:
                    prep_lvl2(n, x, r0, 16, half(when))

            t0 = min(load) + X0 + 32 * XD + 100
            if n >= 2:
                spread('p', job, [(r0, c0) for r0 in range(0, DH // 2, 8) for c0 in (0, T)], t0, t0 + PW)
            else:
                spread('p', job2, [(lvl, x, r0) for lvl in (1, 2) for x in range(1 + 3 * lvl) for r0 in (0, 16)], t0, t0 + PW)

        def side_by_side(dst, w_of, fn, r0, when):
            after = pltpu.bitcast(gate(when - WIN), u32)
            q = {}
            for j in range(2):
                w0, w1 = [lax.select(always, w_of(p, j * dst.shape[1] // 2 + r0), after) for p in range(2)]
                sw = pltpu.roll(lax.select(lo, w1, w0), DH, 1)
                q[0, j], q[1, j] = lax.select(lo, w0, sw), lax.select(lo, sw, w1)
            a = fn([upk(q[i, j]).astype(f32) for i in range(2) for j in range(2)])
            for r in range(7):
                dst[r, 2 * r0:2 * r0 + 16, :] = a[r].astype(bf16)
            toks.append((when + AD, a[4][0:8]))

        pair_weights = functools.partial(side_by_side, a2_s, lambda p, r: wn_s[(slot, 1 - slot)[p], 1 - slot, r:r + 8, :],
                                         lambda x: sum_a(*x))
        kv_weights = functools.partial(side_by_side, akvT_s, lambda p, r: wc_s[p, r:r + 8, :], hsum_a)

        def pair_keep(r, t, when):
            even = lax.select(always, jnp.full((8, T), slot, i32), pltpu.bitcast(gate(when - WIN), i32)) == 0
            no, nq = [pltpu.bitcast(x[r, t], u32).reshape(DH // 16, 8, T) for x in (no_s, nq_s)]
            np_s[r, t] = jnp.where(even, nq, no).reshape(DH // 2, T)

        def stage(st_ref, prev_ref, r0, cur):
            n = cur.shape[0]
            st_ref.at[slot, r0:r0 + n][...] = hcat(prev_ref[r0:r0 + n, :], cur).reshape(n, 2, D)
            prev_ref[r0:r0 + n, :] = cur

        def dw_top(h_s):
            d11, d12, d21, d22 = comb_a([h_s[r] for r in range(7)])
            return xpose(vcat(hcat(d11, d12), hcat(d21, d22)).astype(bf16))

        def kv_fin(which, j2, i2, r0, when):
            o = i2 * DQ + r0
            d = hcomb_a(gated([f1_s[r, 2 * i2 + j2, which * DQ + r0:which * DQ + r0 + 16, :] for r in range(7)], (0, 4, 5), when))
            for x in range(4):
                dwT_s[which, 2 * (x % 2) + j2, (x // 2) * DH + o:(x // 2) * DH + o + 16, :] = d[x].astype(bf16)
            if o == DH - 16:
                def flip():
                    for j in (j2, 2 + j2):
                        stage((stk, stv)[which], (dwk_s, dwv_s)[which], j * T, xpose_at(dwT_s[which, j], when + XL))

                tasks.append((when + XL, 'X', flip))

        def outer(i, r0, when):
            first = lax.select(always, act_s[i, 0], gate(when - WIN))
            rhs = vcat(first[None], act_s[i, 1:C])
            y = jnp.sum(lb_s[i // 2, :, r0:r0 + WR, :].reshape(C, WR // 8, 8, T) * rhs[:, None], axis=0)
            hout[slot, 1 + i, r0:r0 + WR, :] = y.reshape(WR, T).astype(bf16)
            due(when, y[0])

        mt = [slice(m0, min(m0 + T, M)) for m0 in range(0, M, T)]

        def act():
            if 'act' not in ffn:
                ffn['act'] = ffn_act(ffn[0], ffn[1], ffn[2])
            return ffn['act']

        for name in steps:
            assert times[name] == min(load)
            op, args = name[0], [int(x) for x in name[1:].split('.') if x]
            n = args[0] if args else 0
            now = min(load)
            if op == 'L':
                latent(*args)
            elif op in 'QOadp':
                dict(Q=qproj, O=doproj, a=a_, d=d_, p=prep)[op](n)
            elif op in 'cmvn':
                assert op != 'c' or done('e%d' % n)
                dict(c=c_, m=m_, v=v_, n=n_)[op](*args)
            elif op == 'e':
                skip = EF * (2 * n * T + MARG) // 100 if n <= EN else 0
                e_(n, max(now + skip, st['aend', 2 * n], st['aend', 2 * n + 1]) + B0, min(times['c%d.0' % n], times.get('a%d' % (2 * n - 3), 10 ** 9)) - B1)
            elif op == 'T':
                spread('T', kv_weights, [(r0,) for r0 in range(0, KH // 2, 8)], now + T0, now + T0 + TW)
            elif op == 'A':
                spread('A', pair_weights, [(r0,) for r0 in range(0, MH // 2, 8)], now + A0, now + A0 + AW)
            elif op == 'M':
                t0, t1 = now + M0, times['k%d.0' % MK] - M1
                for r in range(7):
                    spread('M%d' % r, dkv2, [(r, b, w, r0) for b in range(NQ - 1, -1, -1) for w in (1, 0) for r0 in (0, 16)],
                           t0 + (t1 - t0) * r // 7, t0 + (t1 - t0) * (r + 1) // 7)
            elif op == 'N':
                spread('N', pair_keep, [(r, t) for r in range(7) for t in range(NB)], now, now + NW)
            elif op == 'o':
                if n < 7:
                    ho_s[z + n] = mm(cat(no_s, range(NB), n), upk(cat(bg_s, range(NB), n)), NT)
                else:
                    hout[slot, 0, 2 * KH:M, :] = mm(gr_s[...], cat(ctxT_s, range(NTL)), NT).astype(bf16)
                    hout[slot, 0, 0:2 * KH, :] = dw_top(ho_s)
            elif op == 'q':
                if n < 7:
                    hq_s[z + n] = mm(cat(nq_s, range(NB), n), upk(cat(bx_s, range(NB), n)), NT)
                else:
                    stage(stq, dwq_s, 2 * KH, mm(xr_s[...], cat(dqT_s, range(NTL)), NT).astype(bf16))
                    stage(stq, dwq_s, 0, dw_top(hq_s))
            elif op == 'k':
                assert done('M%d' % n)
                for r2 in (range(4), range(4, 7))[args[1]]:
                    st['k', r2] = mm(cat(n2_s, range(NQ), 7 * n + r2), upk(cat(b2_s, range(NQ), 7 * n + r2)), NT)
                if args[1]:
                    for x, y in enumerate(hcomb_a([st.pop(('k', r2)) for r2 in range(7)])):
                        f1_s[z + n, x] = y
                if name == 'k6.1':
                    spread('K', kv_fin, [(w, j2, i2, r0) for w in range(2) for j2 in range(2) for i2 in range(2) for r0 in (0, 16)],
                           min(load) + K0, min(min(load) + K0 + KW, times['end'] - K1))
            elif op in 'yg':
                r, ts = n // 2, range(4 * (n % 2), 4 * (n % 2) + 4)
                sp = slice(ts[0] * T, (ts[-1] + 1) * T)
                m = MH if op == 'y' else KH
                rr = slice(0, m) if len(args) == 1 else slice(args[1] * m // 2, (args[1] + 1) * m // 2)
                if op == 'g':
                    assert done('T')
                    gc_a[r, rr, sp] = jnp.where(h >= 1, gc_a[r, rr, sp], 0.0) + mm(akvT_s[r, rr], cat(nkv_s, ts, r))
                else:
                    assert done('A')
                    no, nq = pltpu.bitcast(cat(no_s, ts, r), u32), pltpu.bitcast(cat(nq_s, ts, r), u32)
                    rhs = upk(vcat(jnp.where(slot == 0, no, nq), cat(np_s, ts, r)))
                    g2_a[1 - slot, r, rr, sp] = jnp.where(h >= 2, g2_a[1 - slot, r, rr, sp], 0.0) + mm(a2_s[r, rr], rhs)
            elif op == 'f':
                for i, m in [(i, m) for i in range(3) for m in mt][4 * n:4 * n + 4]:
                    y = mm((xs_s, xs_s, dy_s)[i][:, m], hin[slot, i, m, :])
                    ffn[i] = y if i not in ffn else ffn[i] + y
            elif op == 'b':
                for i, m in [(i, m) for m in mt for i in range(3)][4 * n:4 * n + 4]:
                    (dxs_a, dxs_a, y_a)[i][:, m] += mm(act()[i].astype(bf16), hin[slot, i, m, :], NT)
            elif op == 'W':
                for i in range(3):
                    for c in range(C):
                        act_s[i, c] = jnp.broadcast_to(act()[i][c:c + 1, :], (8, T))
                spread('W', outer, [(i, r0) for i in range(3) for r0 in range(0, M, WR)], now + W0, times['end'] - W1)
        run_tasks(10 ** 9)
        return carry

    lax.fori_loop(jnp.maximum((g - 1) * (HR // NG) - 1, 0), jnp.where(g == NG, HR, g * (HR // NG) - 1), head, 0)

    @pl.when(g == NG)
    def _():
        for cp in cps_hout(HR - 2, 0):
            cp.wait()
        for cp in cps_hout(HR - 1, 1):
            cp.start()
        y = y_a[0:C, :]
        dr = jnp.sum(dy_s[...].astype(f32)[0:C, :] * y, axis=1, keepdims=True) * (1.0 - rs_s[0:C, 0:1])
        dwr_ref[...] = jnp.sum(dr * xs_s[...].astype(f32)[0:C, :], axis=0, keepdims=True).astype(bf16).reshape(M)
        de = dxs_a[0:C, :] + dr * wr_ref[...].reshape(1, M).astype(f32)
        yh, deh = rb(y), rb(de)
        selT_s[...] = vcat(yh, y - yh, deh, de - deh, jnp.zeros((T - 4 * C, M), f32)).astype(bf16).T

        def body(i, carry):
            cols = blk(i)
            oh = oh_s[:, cols]
            zero = jnp.zeros((CP, TB), bf16)
            halves = lambda lhs, rhs: vcat(*[dot(lhs(r0), rhs) for r0 in (0, MH)])
            sel = lambda r0: selT_s[r0:r0 + MH, 0:2 * CP]
            de_ = halves(sel, vcat(zero, oh))
            y_ = halves(sel, vcat(oh, zero)) + halves(
                lambda r0: upk(wn_s[1, 1, r0 // 2:(r0 + MH) // 2, :]), hcat(ctxT_s[2 * i], ctxT_s[2 * i + 1]))
            z = z_s[0]

            def acc(which, r0):
                b11, b12, b21, b22 = comb_b([g2_a[which, r, r0:r0 + RC, tl(i)] for r in range(7)])
                return (r0, hcat(b11, b12)), (MH + r0, hcat(b21, b22))

            s1 = s2 = None
            for r in range(0, MH, RC):
                for r0, a in acc(0, r):
                    dn = a + de_[r0:r0 + RC] + gT_s[r0:r0 + RC, cols].astype(f32)
                    dn_s[z, r0:r0 + RC, :] = dn
                    t = (dn * xnT_s[r0:r0 + RC, cols].astype(f32)).reshape(RC // 8, 8, TB)
                    a1, a2 = jnp.sum(dn.reshape(RC // 8, 8, TB), axis=0), jnp.sum(t, axis=0)
                    s1, s2 = (a1, a2) if s1 is None else (s1 + a1, s2 + a2)
            rstd = stat_s[2, :, cols]
            m1 = jnp.sum(s1, axis=0, keepdims=True) * (rstd * (1.0 / M))
            m2 = jnp.sum(s2, axis=0, keepdims=True) * (rstd * (1.0 / M))
            b11, b12, b21, b22 = hcomb_b([gc_a[r, :, tl(i)] for r in range(7)])
            c_s[cols, :] = vcat(hcat(b11, b12), hcat(b21, b22)).astype(bf16).T
            cols2 = blk(i + z)
            for r in range(0, MH, RC):
                for r0, a in acc(1, r):
                    xh = xnT_s[r0:r0 + RC, cols2].astype(f32)
                    xT_s[r0:r0 + RC, cols] = (a + y_[r0:r0 + RC] + xh + xT_s[r0:r0 + RC, cols].astype(f32)).astype(bf16)
                    dxT = (gT_s[r0:r0 + RC, cols2].astype(f32) - m1) + (dn_s[0, r0:r0 + RC, :] * rstd - xh * m2)
                    gT_s[r0:r0 + RC, cols2] = dxT.astype(bf16)
            cp_dc(i).start()
            cp_out(i).start()
            cp_dx(i).start()
            return carry

        lax.fori_loop(0, NB, body, 0)
        for cp in cps_hout(HR - 1, 1) + cps_xout:
            cp.wait()
        for i in range(NB):
            cp_dc(i).wait()
            cp_out(i).wait()
            cp_dx(i).wait()

  return kernel


def build(NOBC=True, **kw):
  kernel = make_kernel(**kw)

  @jax.jit
  def fn(A_x, A_c_kv, A_w_q, A_w_uk, A_w_uv, A_w_o, B_x, B_w_r, B_w_gate, B_w_up, B_w_down, grad_out):
    hbm = pl.BlockSpec(memory_space=pl.ANY)
    grp = lambda n: pl.BlockSpec((n, HG, D), lambda g: (0, jnp.maximum(g - 1, 0), 0))
    vec = pl.BlockSpec((M,), lambda g: (0,))
    in_specs = [hbm, hbm, hbm, grp(M), grp(DC), grp(DC), hbm, vec, hbm, hbm, hbm]
    out_specs = [hbm, hbm, hbm, hbm, hbm, hbm, hbm, vec, hbm, hbm, hbm]
    sds = lambda *s: jax.ShapeDtypeStruct(s, bf16)
    out_shape = [sds(M, S), sds(M, S), sds(S, DC), sds(M, H // 2, 2, D), sds(DC, H // 2, 2, D), sds(DC, H // 2, 2, D),
                 sds(H, M, D), sds(M), sds(M, F), sds(M, F), sds(M, F)]
    B = lambda *s: pltpu.VMEM(s, bf16)
    R = lambda *s: pltpu.VMEM(s, f32)
    P = lambda *s: pltpu.VMEM(s[:-2] + (s[-2] // 2, s[-1]), u32)
    DMA = pltpu.SemaphoreType.DMA
    NOFF = NB * (NB - 1) // 2
    scratch = [
        B(M, S), B(M, S), B(M, S), B(S, DC), P(7, NB, KH, T), P(7, NB, KH, T), P(49, NQ, T, T), P(MR, S), P(MR, S),
        R(3, 1, S), R(1, S), R(2, 7, MH, S // 2), R(7, KH, S // 2),
        B(M, HG * D), B(2, DC, HG * D), P(2, 2, M, D), P(2, DC, D), P(4, D, 2 * KH), P(7, DH, KH), P(7, DH, KH), P(49, DH, T),
        B(D, MR), B(D, MR), B(7, KH, D), B(7, MH, D),
        B(NTL, D, T), P(1, S, D), B(NTL, D, T), P(1, S, D), B(NTL, D, T), B(NTL, D, T), B(NTL, D, T), B(NTL, D, T),
        B(7, NB, DH, T), B(7, NB, DH, T), B(7, NB, DH, T), B(7, NB, DH, T), B(7, NB, DH, T), B(7, NB, DH, T),
        P(7, NB, DH, T), B(7, NB, D, T),
        pltpu.SMEM((1,), i32), R(1, NTL, T, T), R(1, NTL, T, T), R(1, NTL, T, T), R(1, NTL, T, T),
        B(NTL * (NTL + 1) // 2, T, T), B(5, NOFF, T, T), B(7, NOFF, T, T), B(NB, 3, T, T),
        R(7, DH, KH), R(7, DH, KH), R(7, 4, DH, T), R(7, 4, DH, T), R(7, 4, DH, T), B(49, NQ, DH, T), B(2, 4, D, T),
        B(M, D), B(DC, D), B(DC, D),
        R(M, T), R(C, S), R(C, S), B(CP, S), R(M, T), B(M, T), B(CP, M), B(CP, M), R(CP, T), R(2, C, M, T), R(3, C, 8, T),
        R(CP, M), R(CP, M), R(1, M, TB), P(1, DC, 4 * T),
        B(2, 4, M, T), B(2, 4, M, T), B(2, M, 2, D), B(2, DC, 2, D), B(2, DC, 2, D), B(3, M, FX), B(3, M, FX),
        DMA((NB,)), DMA((NB,)), DMA((NB,)), DMA((1,)), DMA((1,)), DMA((1,)), DMA((1,)), DMA((1,)),
    ]
    outs = pl.pallas_call(
        kernel, grid=(NG + 1,), in_specs=in_specs, out_specs=out_specs, out_shape=out_shape, scratch_shapes=scratch,
        compiler_params=pltpu.CompilerParams(dimension_semantics=("arbitrary",), vmem_limit_bytes=126 * 2 ** 20,
                                             disable_bounds_checks=NOBC),
        name="fused_kernel",
    )(A_x.reshape(S, M).T, A_c_kv.reshape(S, DC), grad_out.reshape(S, M).T, A_w_q, A_w_uk, A_w_uv, A_w_o.transpose(0, 2, 1),
      B_w_r, B_w_gate, B_w_up, B_w_down.T)
    out, dx, dc, dwq, dwuk, dwuv, dwo, dwr, dwg, dwu, dwd = outs
    return (out.T.reshape(1, S, M), dx.T.reshape(1, S, M), dc.reshape(1, S, DC), dwq.reshape(M, H, D), dwuk.reshape(DC, H, D),
            dwuv.reshape(DC, H, D), dwo.transpose(0, 2, 1), dwr, dwg, dwu, dwd.T)

  return fn


_fn = build(XL=250)


@jax.jit
def pallas_parallel_sum__compressed_kv_cla__moe_arch_mod__prompt_kernel(
    A_x: jax.Array,
    A_c_kv: jax.Array,
    A_w_q: jax.Array,
    A_w_uk: jax.Array,
    A_w_uv: jax.Array,
    A_w_o: jax.Array,
    B_x: jax.Array,
    B_w_r: jax.Array,
    B_w_gate: jax.Array,
    B_w_up: jax.Array,
    B_w_down: jax.Array,
    grad_out: jax.Array,
):
    return _fn(A_x, A_c_kv, A_w_q, A_w_uk, A_w_uv, A_w_o, B_x, B_w_r, B_w_gate, B_w_up, B_w_down, grad_out)
```
